```python
import jax
import jax.numpy as jnp

def _softmax(x, axis=-1):
    return jax.nn.softmax(x, axis=axis)
def _gelu(x):
    return jax.nn.gelu(x, approximate=True)
def _silu(x):
    return jax.nn.silu(x)
def _sigmoid(x):
    return jax.nn.sigmoid(x)
def _layernorm(x, axis=-1, eps=1e-5):
    m = jnp.mean(x, axis=axis, keepdims=True)
    v = jnp.var(x, axis=axis, keepdims=True)
    return (x - m) / jnp.sqrt(v + eps)
def _scatter_add(tgt, idx, src, axis=0):
    return tgt.at[idx].add(src)
def _segment_sum(src, seg, n):
    return jax.ops.segment_sum(src, seg, n)
class _Rng:
    def __init__(self, key):
        self._k = key
    def _next(self):
        self._k, sub = jax.random.split(self._k)
        return sub
    def normal(self, shape):
        return jax.random.normal(self._next(), shape, dtype=jnp.bfloat16)
    def randint(self, lo, hi, shape):
        return jax.random.randint(self._next(), shape, lo, hi, dtype=jnp.int32)
    def uniform(self, shape, lo=0.0, hi=1.0):
        return jax.random.uniform(self._next(), shape, jnp.bfloat16, lo, hi)
    def permutation(self, n):
        return jax.random.permutation(self._next(), n)


kernel_name = 'gated_mix__compressed_kv_cla__sliding_block_cached__decode'

def setup_inputs():
    _rng = _Rng(jax.random.key(int.from_bytes(__import__("os").urandom(4), "little")))
    _w = (lambda a: (lambda t: t.astype(jnp.bfloat16) if jnp.issubdtype(t.dtype, jnp.floating) else t)(jnp.asarray(a)))
    def _A_setup():
        B, H, Sq, Sk, D, M = 8, 32, 1, 4096, 128, 512
        Dc = 4 * D
        return {
            "x": _w((lambda *s: _rng.normal(s) * 0.05)(B, Sq, M)),
            "c_kv": _w((lambda *s: _rng.normal(s) * 0.05)(B, Sk, Dc)),
            "w_q": _w((lambda *s: _rng.normal(s) * 0.05)(M, H, D) * (M ** -0.5)),
            "w_uk": _w((lambda *s: _rng.normal(s) * 0.05)(Dc, H, D) * (Dc ** -0.5)),
            "w_uv": _w((lambda *s: _rng.normal(s) * 0.05)(Dc, H, D) * (Dc ** -0.5)),
            "w_o": _w((lambda *s: _rng.normal(s) * 0.05)(H, D, M) * ((H * D) ** -0.5)),
        }
    _A_in = _A_setup()

    def _B_setup():
        B, Sq, D = 8, 1, 512
        Hq, Hkv, Sk, Dh = 32, 8, 4096, 128
        assert Hq % Hkv == 0, (Hq, Hkv)
        return {
            "x": _w((lambda *s: _rng.normal(s) * 0.05)(B, Sq, D)),
            "k_cache": _w((lambda *s: _rng.normal(s) * 0.05)(B, Hkv, Sk, Dh)),
            "v_cache": _w((lambda *s: _rng.normal(s) * 0.05)(B, Hkv, Sk, Dh)),
            "wq": _w((lambda *s: _rng.normal(s) * 0.05)(D, Hq * Dh) * (D ** -0.5)),
            "wo": _w((lambda *s: _rng.normal(s) * 0.05)(Hq * Dh, D) * ((Hq * Dh) ** -0.5)),
        }
    _B_in = _B_setup()

    return {
        "A_x": _A_in["x"],
        "A_c_kv": _A_in["c_kv"],
        "A_w_q": _A_in["w_q"],
        "A_w_uk": _A_in["w_uk"],
        "A_w_uv": _A_in["w_uv"],
        "A_w_o": _A_in["w_o"],
        "B_x": _B_in["x"],
        "B_k_cache": _B_in["k_cache"],
        "B_v_cache": _B_in["v_cache"],
        "B_wq": _B_in["wq"],
        "B_wo": _B_in["wo"],
        "gate_w": _w((lambda *s: _rng.normal(s) * 0.05)(512)),
    }

def reference(A_x, A_c_kv, A_w_q, A_w_uk, A_w_uv, A_w_o, B_x, B_k_cache, B_v_cache, B_wq, B_wo, gate_w):
    def _A_ref(x, c_kv, w_q, w_uk, w_uv, w_o):
        B, Sq, M = x.shape[0], x.shape[1], x.shape[2]
        Sk = c_kv.shape[1]
        H, D = w_q.shape[1], w_q.shape[2]
        q = jnp.einsum("bqm,mhd->bhqd", x, w_q)
        k = jnp.einsum("bkc,chd->bhkd", c_kv, w_uk)
        v = jnp.einsum("bkc,chd->bhkd", c_kv, w_uv)
        scores = jnp.einsum("bhqd,bhkd->bhqk", q, k) * (D ** -0.5)
        off = Sk - Sq
        qi = jnp.arange(Sq)[:, None]
        kj = jnp.arange(Sk)[None, :]
        cmask = kj <= (qi + off)
        scores = jnp.where(cmask[None, None], scores, -1e9)
        p = _softmax(scores, axis=-1)
        ctx = jnp.einsum("bhqk,bhkd->bhqd", p, v)
        return jnp.einsum("bhqd,hdm->bqm", ctx, w_o)

    def _B_ref(x, k_cache, v_cache, wq, wo):
        B, Sq, D = x.shape
        Hq, Dh = 32, 128
        Hkv, Sk = k_cache.shape[1], k_cache.shape[2]
        W = min(4096, max(256, Sk // 4))
        rep = Hq // Hkv
        q = (lambda x, *d: x.transpose(*d))((x @ wq).reshape(B, Sq, Hq, Dh), 0, 2, 1, 3)
        k = jnp.repeat(k_cache[:, :, Sk - W:, :], rep, axis=1)
        v = jnp.repeat(v_cache[:, :, Sk - W:, :], rep, axis=1)
        scores = jnp.einsum("bhqd,bhkd->bhqk", q, k) * (Dh ** -0.5)
        p = _softmax(scores, axis=-1)
        o = jnp.einsum("bhqk,bhkd->bhqd", p, v)
        return (lambda x, *d: x.transpose(*d))(o, 0, 2, 1, 3).reshape(B, Sq, Hq * Dh) @ wo

    x = A_x
    g = _sigmoid((x * gate_w).sum(-1, keepdims=True))
    a = _A_ref(x, A_c_kv, A_w_q, A_w_uk, A_w_uv, A_w_o)
    b = _B_ref(x, B_k_cache, B_v_cache, B_wq, B_wo)
    return g * a + (1 - g) * b
```

```python
import jax
import jax.numpy as jnp
from jax import lax
import jax.experimental.pallas as pl
import jax.experimental.pallas.tpu as pltpu

B = 8
H = 32
D = 128
M = 512
C = 512
SK = 4096
HKV = 8
W = 1024
SCALE = D ** -0.5

NSTREAM = 8
NPIECE = 8
NSEM = 4

F32 = jnp.float32
BF16 = jnp.bfloat16
U32 = jnp.uint32

NN = (((1,), (0,)), ((), ()))
NT = (((1,), (1,)), ((), ()))


def _dot(a, b, dims):
    return lax.dot_general(a, b, dims, preferred_element_type=F32)


def _kernel(x_h, ckv_h, wq_h, wuk_h, wuv_h, wo_h, k_h, v_h, bwq_h, bwo_h, g_h,
            o_ref,
            x_v, g_v, ckv_v, wq_v, wuk_v, wuv_v, wo_v, kv_v, bwq_v, bwo_v,
            qa_s, qabs_s, s_s, lat_s, qb_s, ctxa_s, ctxb_s, sb_s, sems):

    def issue_rows(src, dst, nrows, j, sem):
        per = nrows // NSTREAM
        rpc = nrows // 128
        for i in range(2):
            for s in range(NSTREAM):
                off = pl.multiple_of(s * per + (2 * j + i) * rpc, rpc)
                pltpu.make_async_copy(
                    src.at[pl.ds(off, rpc)], dst.at[pl.ds(off, rpc)], sem
                ).start(priority=s % 2)

    def issue_bwq(j, sem):
        for i in range(2):
            for s in range(NSTREAM):
                off = pl.multiple_of(s * 64 + j * 8, 8)
                pltpu.make_async_copy(
                    bwq_h.at[pl.ds(off, 8), pl.ds(i * 2048, 2048)],
                    bwq_v.at[pl.ds(off, 8), pl.ds(i * 2048, 2048)], sem
                ).start(priority=s % 2)

    def issue_kv(b, j, sem):
        off = pl.multiple_of(j * 128, 128)
        for h in range(HKV):
            pltpu.make_async_copy(
                k_h.at[b, h, pl.ds(SK - W + off, 128)],
                kv_v.at[b, 0, h, pl.ds(off, 128)], sem).start(priority=0)
            pltpu.make_async_copy(
                v_h.at[b, h, pl.ds(SK - W + off, 128)],
                kv_v.at[b, 1, h, pl.ds(off, 128)], sem).start(priority=1)

    def issue_ckv(b, j, sem):
        issue_rows(ckv_h.at[b], ckv_v.at[b], SK, j, sem)

    def wait_unit(buf, sem):
        pltpu.make_async_copy(buf, buf, sem).wait()

    def sem_of(u):
        return sems.at[u % NSEM]

    def loop(n, body):
        def f(i, c):
            body(i)
            return c
        lax.fori_loop(0, n, f, 0)

    U_WQ, U_WUK, U_CKV, U_BWQ, U_WUV, U_KV, U_WO, U_BWO = 0, 1, 2, 10, 11, 12, 20, 21

    cx = pltpu.make_async_copy(x_h, x_v, sems.at[3])
    cg = pltpu.make_async_copy(g_h, g_v, sems.at[3])
    cx.start()
    cg.start()
    loop(NPIECE, lambda j: issue_rows(wq_h, wq_v, M * H, j, sem_of(U_WQ)))
    loop(NPIECE, lambda j: issue_rows(wuk_h, wuk_v, C * H, j, sem_of(U_WUK)))
    cx.wait()
    cg.wait()

    def head_pair(w_v, g, t):
        w32 = w_v.bitcast(U32).at[pl.ds(pl.multiple_of(4 * g, 4), 8180)]
        a = w32[pl.ds(t, 256, stride=32), :]
        b = w32[pl.ds(t + 16, 256, stride=32), :]
        w0 = pltpu.bitcast((a & U32(0xFFFF)) | (b << 16), BF16)
        w1 = pltpu.bitcast((a >> 16) | (b & U32(0xFFFF0000)), BF16)
        return w0, w1

    def head_rows(ref, g):
        return ref.at[pl.ds(pl.multiple_of(8 * g, 8), B * H - 24)]

    def weight_unit(w_v, u, issue, per_head):
        def step(g):
            for t in range(4):
                if t % 2 == 0:
                    issue(2 * g + t // 2)
                if t == 0:
                    @pl.when(g == 0)
                    def _():
                        wait_unit(w_v, sem_of(u))
                ws = head_pair(w_v, g, t)
                per_head(g, 2 * t, ws[0])
                per_head(g, 2 * t + 1, ws[1])
        loop(4, step)

    def wq_head(g, e, w):
        r = pl.multiple_of(g * 64 + e * 8, 8)
        qa_s[pl.ds(r, 8), :] = _dot(x_v[...], w, NN)
    weight_unit(wq_v, U_WQ, lambda j: issue_ckv(0, j, sem_of(U_CKV)), wq_head)

    def wuk_head(g, e, w):
        r = pl.multiple_of(g * 64 + e * 8, 8)
        q = qa_s[pl.ds(r, 8), :].astype(BF16)
        qa = _dot(q, w, NT) * SCALE
        for ct in range(4):
            head_rows(qabs_s.at[ct], g)[pl.ds(e, B, stride=H), :] = (
                qa[:, ct * 128:(ct + 1) * 128])
    weight_unit(wuk_v, U_WUK, lambda j: issue_ckv(1, j, sem_of(U_CKV + 1)), wuk_head)

    def ckv_unit(b):
        u = U_CKV + b

        def issue(j):
            sem = sem_of(u + 2)

            @pl.when(b < B - 2)
            def _():
                issue_ckv(jnp.minimum(b + 2, B - 1), j, sem)

            @pl.when(b == B - 2)
            def _():
                issue_bwq(j, sem)

            @pl.when(b == B - 1)
            def _():
                issue_rows(wuv_h, wuv_v, C * H, j, sem)

        issue(0)
        wait_unit(ckv_v.at[b], sem_of(u))
        r = pl.multiple_of(b * H, H)
        qa = jnp.concatenate(
            [qabs_s[ct, pl.ds(r, H), :] for ct in range(4)], axis=1
        ).astype(BF16)
        KC = SK // 4

        def score_step(j, m):
            @pl.when(j > 0)
            def _():
                issue(j)
            off = pl.multiple_of(j * KC, KC)
            s = _dot(qa, ckv_v[b, pl.ds(off, KC), :], NT)
            s_s[j] = s
            for t in range(KC // 128):
                m = jnp.maximum(m, s[:, t * 128:(t + 1) * 128])
            return m
        m = lax.fori_loop(0, 4, score_step, jnp.full((H, 128), -jnp.inf, F32))
        m = jnp.max(m, axis=1, keepdims=True)

        def pv_step(j, carry):
            l, acc = carry
            issue(4 + j)
            off = pl.multiple_of(j * KC, KC)
            p = jnp.exp(s_s[j] - m)
            for t in range(KC // 128):
                l = l + p[:, t * 128:(t + 1) * 128]
            acc = acc + _dot(p.astype(BF16), ckv_v[b, pl.ds(off, KC), :], NN)
            return l, acc
        l, acc = lax.fori_loop(
            0, 4, pv_step, (jnp.zeros((H, 128), F32), jnp.zeros((H, C), F32)))
        lat = acc / jnp.sum(l, axis=1, keepdims=True)
        for ct in range(4):
            lat_s[ct, pl.ds(r, H), :] = lat[:, ct * 128:(ct + 1) * 128]
    loop(B, ckv_unit)

    def bwq_step(g):
        for t in range(2):
            issue_kv(0, 2 * g + t, sem_of(U_KV))
            if t == 0:
                @pl.when(g == 0)
                def _():
                    wait_unit(bwq_v, sem_of(U_BWQ))
            off = pl.multiple_of(g * 1024 + t * 512, 512)
            q = _dot(x_v[...], bwq_v[:, pl.ds(off, 512)], NN)
            for e in range(4):
                head_rows(qb_s, g)[pl.ds(4 * t + e, B, stride=H), :] = (
                    q[:, e * 128:(e + 1) * 128])
    loop(4, bwq_step)

    def wuv_head(g, e, w):
        lat = jnp.concatenate(
            [head_rows(lat_s.at[ct], g)[pl.ds(e, B, stride=H), :]
             for ct in range(4)], axis=1).astype(BF16)
        r = pl.multiple_of(g * 64 + e * 8, 8)
        ctxa_s[pl.ds(r, 8), :] = _dot(lat, w, NN)
    weight_unit(wuv_v, U_WUV, lambda j: issue_kv(1, j, sem_of(U_KV + 1)), wuv_head)

    def kv_unit(b):
        u = U_KV + b

        def issue(j):
            sem = sem_of(u + 2)

            @pl.when(b < B - 2)
            def _():
                issue_kv(jnp.minimum(b + 2, B - 1), j, sem)

            @pl.when(b == B - 2)
            def _():
                issue_rows(wo_h, wo_v, H * D, j, sem)

            @pl.when(b == B - 1)
            def _():
                issue_rows(bwo_h, bwo_v, H * D, j, sem)

        def pair_step(i):
            issue(2 * i)

            @pl.when(i == 0)
            def _():
                wait_unit(kv_v.at[b], sem_of(u))
            r = pl.multiple_of(b * H + i * 8, 8)
            q = qb_s[pl.ds(r, 8), :].astype(BF16)
            lo = lax.broadcasted_iota(jnp.int32, (8, W), 0) < 4
            s0 = _dot(q, kv_v[b, 0, 2 * i], NT)
            s1 = _dot(q, kv_v[b, 0, 2 * i + 1], NT)
            s = jnp.where(lo, s0, s1) * SCALE
            sb_s[...] = s - jnp.max(s, axis=1, keepdims=True)
            issue(2 * i + 1)
            p = jnp.exp(sb_s[...])
            l = jnp.sum(p, axis=1, keepdims=True)
            pb = p.astype(BF16)
            o0 = _dot(pb, kv_v[b, 1, 2 * i], NN)
            o1 = _dot(pb, kv_v[b, 1, 2 * i + 1], NN)
            lo = lax.broadcasted_iota(jnp.int32, (8, D), 0) < 4
            o = jnp.where(lo, o0, o1) / l
            ctxb_s[pl.ds(r, 8), :] = o
        loop(4, pair_step)
    loop(B, kv_unit)

    x = x_v[...].astype(F32)
    gw = g_v[...].astype(F32).reshape(1, M)
    g = jax.nn.sigmoid(jnp.sum(x * gw, axis=1, keepdims=True))
    ctxa = jnp.concatenate(
        [ctxa_s[h * 8:(h + 1) * 8, :] for h in range(H)], axis=1).astype(BF16)
    ctxb = jnp.concatenate(
        [ctxb_s[pl.ds(h, B, stride=H), :] for h in range(H)], axis=1).astype(BF16)
    wait_unit(wo_v, sem_of(U_WO))
    a = _dot(ctxa, wo_v[...], NN)
    wait_unit(bwo_v, sem_of(U_BWO))
    bb = _dot(ctxb, bwo_v[...], NN)
    o_ref[...] = (g * a + (1.0 - g) * bb).astype(o_ref.dtype)


@jax.jit
def pallas_gated_mix__compressed_kv_cla__sliding_block_cached__decode_kernel(
    A_x: jax.Array,
    A_c_kv: jax.Array,
    A_w_q: jax.Array,
    A_w_uk: jax.Array,
    A_w_uv: jax.Array,
    A_w_o: jax.Array,
    B_x: jax.Array,
    B_k_cache: jax.Array,
    B_v_cache: jax.Array,
    B_wq: jax.Array,
    B_wo: jax.Array,
    gate_w: jax.Array,
):
    del B_x
    hbm = pl.BlockSpec(memory_space=pl.ANY)
    out = pl.pallas_call(
        _kernel,
        out_shape=jax.ShapeDtypeStruct((B, M), A_x.dtype),
        in_specs=[hbm] * 11,
        out_specs=pl.BlockSpec(memory_space=pltpu.VMEM),
        scratch_shapes=[
            pltpu.VMEM((B, M), BF16),
            pltpu.VMEM((M,), BF16),
            pltpu.VMEM((B, SK, C), BF16),
            pltpu.VMEM((M * H, D), BF16),
            pltpu.VMEM((C * H, D), BF16),
            pltpu.VMEM((C * H, D), BF16),
            pltpu.VMEM((H * D, M), BF16),
            pltpu.VMEM((B, 2, HKV, W, D), BF16),
            pltpu.VMEM((M, H * D), BF16),
            pltpu.VMEM((H * D, M), BF16),
            pltpu.VMEM((H * B, D), F32),
            pltpu.VMEM((4, H * B, 128), F32),
            pltpu.VMEM((4, H, SK // 4), F32),
            pltpu.VMEM((4, B * H, 128), F32),
            pltpu.VMEM((H * B, D), F32),
            pltpu.VMEM((H * B, D), F32),
            pltpu.VMEM((B * H, D), F32),
            pltpu.VMEM((8, W), F32),
            pltpu.SemaphoreType.DMA((NSEM,)),
        ],
        compiler_params=pltpu.CompilerParams(
            vmem_limit_bytes=100 * 1024 * 1024,
        ),
    )(
        A_x.reshape(B, M), A_c_kv,
        A_w_q.reshape(M * H, D), A_w_uk.reshape(C * H, D), A_w_uv.reshape(C * H, D),
        A_w_o.reshape(H * D, M), B_k_cache, B_v_cache, B_wq, B_wo, gate_w,
    )
    return out.reshape(B, 1, M)
```

```python
import jax
import jax.numpy as jnp
from jax import lax
import jax.experimental.pallas as pl
import jax.experimental.pallas.tpu as pltpu

B = 8
H = 32
D = 128
M = 512
C = 512
SK = 4096
HKV = 8
W = 1024
SCALE = D ** -0.5

NPIECE = 8
NRING = 4
NSEM = NRING + 4

REM_W = 8
REM_CKV = 0
REM_BWO = 8
REM_KV = 40
REM_BWQ = 5

KV_HEADS = (0, 1, 2, 3, 4, 5, 6, 7)
SPLIT = 2
PAT = (16, 64)
SKIP = ()
BENCH = None
F32 = jnp.float32
BF16 = jnp.bfloat16
U32 = jnp.uint32

NN = (((1,), (0,)), ((), ()))
NT = (((1,), (1,)), ((), ()))


def _dot(a, b, dims):
    return lax.dot_general(a, b, dims, preferred_element_type=F32)


def _kernel(x_h, ckv_h, wq_h, wuk_h, wuv_h, wo_h, k_h, v_h, bwq_h, bwo_h, g_h,
            o_ref,
            x_v, g_v, ckv_v, wq_v, wuk_v, wuv_v, wo_v, kv_v, bwq_v, bwo_v,
            qa_s, qabs_s, s_s, lat_s, qb_s, ctxa_s, ctxb_s, sb_s, sems):

    def chunk_bits(i):
        b1 = (i >> 1) & 1
        return (i & 1) * PAT[0] + b1 * 32 + ((i >> 2) & 1) * PAT[1] + (i >> 3), b1

    def copy(src, dst, sem, prio):
        pltpu.make_async_copy(src, dst, sem).start(priority=prio)

    def issue_rows(src, dst, nrows, rem, j, sem):
        rpc = nrows // 128
        align = 8 if rem else rpc
        jx = (j, j ^ 1)
        for i in range(16):
            hi, b1 = chunk_bits(i)
            start = (hi + 1) * rpc + rem + jx[b1] * (2 * rpc)
            if i == 15:
                start = jnp.where(j == 6, rem, start)
            sm = sem(i) if callable(sem) else sem

            def go(r, r0, n, i=i, b1=b1, sm=sm):
                d = dst(i, jx[b1], r0, n) if callable(dst) else dst.at[pl.ds(r, n)]
                copy(src.at[pl.ds(r, n)], d, sm, i % 2)

            if i == 7 and rem:
                @pl.when(j == 6)
                def _():
                    go(nrows - rpc + rem, 0, rpc - rem)
                    go(0, rpc - rem, rem)

                @pl.when(j != 6)
                def _():
                    go(pl.multiple_of(start, align), 0, rpc)
            else:
                go(pl.multiple_of(start, align), 0, rpc)

    def issue_bwq(j, sem):
        c0, c1 = REM_BWQ * 128, (REM_BWQ + 16) * 128
        jx = (j, j ^ 1)
        for i in range(16):
            hi, b1 = chunk_bits(i)
            r = pl.multiple_of((hi // 2) * 8 + jx[b1] * 8, 8)
            rn = pl.multiple_of((r + 8) & (M - 1), 8)

            def go(r, c, n, i=i):
                copy(bwq_h.at[pl.ds(r, 8), pl.ds(c, n)],
                     bwq_v.at[pl.ds(r, 8), pl.ds(c, n)], sem, i % 2)

            if i < 8:
                go(r, c1, H * D - c1)
                if c0:
                    go(rn, 0, c0)
            else:
                go(rn, c0, c1 - c0)

    def issue_kv(b, g, t, sem):
        def piece(edge):
            for h in KV_HEADS:
                k = (2 * g + t) ^ (2 * (h & 1))
                start = pl.multiple_of(((k + 1) * 128 + REM_KV) & (W - 1), 8)
                for a, src in enumerate((k_h, v_h)):
                    def go(r, n):
                        copy(src.at[b, h, pl.ds(SK - W + r, n)],
                             kv_v.at[b, a, h, pl.ds(r, n)], sem, a)
                    if edge != h & 1:
                        go(start, 128)
                    elif t == 0:
                        go(W - 128 + REM_KV, 128 - REM_KV)
                    else:
                        go(0, 128 + REM_KV)
        pl.when(g < 2)(lambda: piece(None))
        pl.when(g == 2)(lambda: piece(1))
        pl.when(g == 3)(lambda: piece(0))

    def issue_wide(src, dst, j, sem):
        if not SPLIT:
            return issue_rows(src, dst, 4096, REM_CKV, j, sem)
        jx = (j, j ^ 1)
        for i in range(16):
            hi, b1 = chunk_bits(i)
            r = (hi + 1) * 32 + jx[b1] * 64
            if i == 15:
                r = jnp.where(j == 6, 0, r)
            r = pl.multiple_of(r, 32)

            def go(r, n, c, m, i=i):
                copy(src.at[pl.ds(r, n), pl.ds(c, m)],
                     dst.at[pl.ds(r, n), pl.ds(c, m)], sem, i % 2)

            if SPLIT == 2:
                go(r, 32, 128, 384)
                if i in (7, 15):
                    pl.when(j == 6)(
                        (lambda: go(4096 - 24, 24, 0, 128)) if i == 7
                        else (lambda: go(0, 40, 0, 128)))
                    pl.when(j != 6)(lambda: go(r + 8, 32, 0, 128))
                else:
                    go(r + 8, 32, 0, 128)
            else:
                if i == 15:
                    pl.when(j == 6)(lambda: go(0, 8, 0, 128))
                go(r, 8, 128, 384)
                go(r + 8, 24, 0, 512)
                if i == 7:
                    pl.when(j != 6)(lambda: go(r + 32, 8, 0, 128))
                else:
                    go(r + 32, 8, 0, 128)

    def issue_ckv(b, j, sem):
        issue_wide(ckv_h.at[b], ckv_v.at[b], j, sem)

    def issue_bwo(j):
        def dst(i, jj, r0, n):
            s4 = ((i >> 1) & 1) + 2 * ((i >> 2) & 1)
            r = s4 * 128 + (i >> 3) * 32 + (jj & 1) * 64 + r0
            return bwo_v.at[i & 1, jj >> 1, pl.ds(pl.multiple_of(r, 8), n)]

        def sem(i):
            return sems.at[NRING + (j >> 1)] if i & 1 else sem_of(U_BWO)
        issue_rows(bwo_h, dst, H * D, REM_BWO, j, sem)

    def wait_unit(buf, sem, force=False):
        if "waits" in SKIP and not force:
            return
        pltpu.make_async_copy(buf, buf, sem).wait()

    def sem_of(u):
        return sems.at[u % NRING]

    def loop(n, body):
        def f(i, c):
            body(i)
            return c
        lax.fori_loop(0, n, f, 0)

    U_WQ, U_WUK, U_CKV, U_BWQ, U_WUV, U_KV, U_WO, U_BWO = 0, 1, 2, 10, 11, 12, 20, 21

    if BENCH is not None:
        sm = sems.at[0]
        n = 0
        for w in BENCH:
            if w in ("wq", "wuk", "wuv"):
                hh, vv = dict(wq=(wq_h, wq_v), wuk=(wuk_h, wuk_v), wuv=(wuv_h, wuv_v))[w]
                loop(8, lambda j: issue_rows(hh, vv, M * H, REM_W, j, sm)); n += 1
            elif w == "wo":
                loop(8, lambda j: issue_wide(wo_h, wo_v, j, sm)); n += 1
            elif w == "bwo":
                loop(8, lambda j: issue_rows(bwo_h, wo_v, H * D, REM_BWO, j, sm)); n += 1
            elif w == "bwq":
                loop(8, lambda j: issue_bwq(j, sm)); n += 1
            elif w == "ckv":
                loop(8, lambda b: loop(8, lambda j: issue_ckv(b, j, sm))); n += 8
            elif w == "kv":
                def f(b, g):
                    issue_kv(b, g, 0, sm)
                    issue_kv(b, g, 1, sm)
                loop(8, lambda b: loop(4, lambda g: f(b, g))); n += 8
        for _ in range(n):
            wait_unit(wo_v, sm, True)
        o_ref[...] = jnp.zeros_like(o_ref)
        return

    cx = pltpu.make_async_copy(x_h, x_v, sems.at[3])
    cg = pltpu.make_async_copy(g_h, g_v, sems.at[3])
    cx.start()
    cg.start()
    loop(NPIECE, lambda j: issue_rows(wq_h, wq_v, M * H, REM_W, j, sem_of(U_WQ)))
    loop(NPIECE, lambda j: issue_rows(wuk_h, wuk_v, C * H, REM_W, j, sem_of(U_WUK)))
    cx.wait()
    cg.wait()

    def head_pair(w_v, g, t):
        w32 = w_v.bitcast(U32).at[pl.ds(pl.multiple_of(4 * g, 4), 8180)]
        a = w32[pl.ds(t, 256, stride=32), :]
        b = w32[pl.ds(t + 16, 256, stride=32), :]
        w0 = pltpu.bitcast((a & U32(0xFFFF)) | (b << 16), BF16)
        w1 = pltpu.bitcast((a >> 16) | (b & U32(0xFFFF0000)), BF16)
        return w0, w1

    def head_rows(ref, g):
        return ref.at[pl.ds(pl.multiple_of(8 * g, 8), B * H - 24)]

    def weight_unit(w_v, u, issue, per_head):
        def step(g):
            for t in range(4):
                if t % 2 == 0:
                    issue(g, t // 2)
                if t == 0:
                    @pl.when(g == 0)
                    def _():
                        wait_unit(w_v, sem_of(u))
                if "w" in SKIP:
                    continue
                ws = head_pair(w_v, g, t)
                per_head(g, 2 * t, ws[0])
                per_head(g, 2 * t + 1, ws[1])
        loop(4, step)

    def wq_head(g, e, w):
        r = pl.multiple_of(g * 64 + e * 8, 8)
        qa_s[pl.ds(r, 8), :] = _dot(x_v[...], w, NN)
    weight_unit(wq_v, U_WQ, lambda g, t: issue_ckv(0, 2 * g + t, sem_of(U_CKV)), wq_head)

    def wuk_head(g, e, w):
        r = pl.multiple_of(g * 64 + e * 8, 8)
        q = qa_s[pl.ds(r, 8), :].astype(BF16)
        qa = _dot(q, w, NT) * SCALE
        for ct in range(4):
            head_rows(qabs_s.at[ct], g)[pl.ds(e, B, stride=H), :] = (
                qa[:, ct * 128:(ct + 1) * 128])
    weight_unit(wuk_v, U_WUK, lambda g, t: issue_ckv(1, 2 * g + t, sem_of(U_CKV + 1)), wuk_head)

    def ckv_unit(b):
        u = U_CKV + b

        def issue(j):
            sem = sem_of(u + 2)

            @pl.when(b < B - 2)
            def _():
                issue_ckv(jnp.minimum(b + 2, B - 1), j, sem)

            @pl.when(b == B - 2)
            def _():
                issue_bwq(j, sem)

            @pl.when(b == B - 1)
            def _():
                issue_rows(wuv_h, wuv_v, C * H, REM_W, j, sem)

        issue(0)
        wait_unit(ckv_v.at[b], sem_of(u))
        r = pl.multiple_of(b * H, H)
        qa = jnp.concatenate(
            [qabs_s[ct, pl.ds(r, H), :] for ct in range(4)], axis=1
        ).astype(BF16)
        KC = SK // 4

        def score_step(j, m):
            @pl.when(j > 0)
            def _():
                issue(j)
            if "ckv" in SKIP:
                return m
            off = pl.multiple_of(j * KC, KC)
            s = _dot(qa, ckv_v[b, pl.ds(off, KC), :], NT)
            s_s[j] = s
            for t in range(KC // 128):
                m = jnp.maximum(m, s[:, t * 128:(t + 1) * 128])
            return m
        m = lax.fori_loop(0, 4, score_step, jnp.full((H, 128), -jnp.inf, F32))
        m = jnp.max(m, axis=1, keepdims=True)

        def pv_step(j, carry):
            l, acc = carry
            issue(4 + j)
            if "ckv" in SKIP:
                return l + s_s[j][:, :128], acc + s_s[j][:, :512]
            off = pl.multiple_of(j * KC, KC)
            p = jnp.exp(s_s[j] - m)
            for t in range(KC // 128):
                l = l + p[:, t * 128:(t + 1) * 128]
            acc = acc + _dot(p.astype(BF16), ckv_v[b, pl.ds(off, KC), :], NN)
            return l, acc
        l, acc = lax.fori_loop(
            0, 4, pv_step, (jnp.zeros((H, 128), F32), jnp.zeros((H, C), F32)))
        lat = acc / jnp.sum(l, axis=1, keepdims=True)
        for ct in range(4):
            lat_s[ct, pl.ds(r, H), :] = lat[:, ct * 128:(ct + 1) * 128]
    loop(B, ckv_unit)

    def bwq_step(g):
        for t in range(2):
            issue_kv(0, g, t, sem_of(U_KV))
            if t == 0:
                @pl.when(g == 0)
                def _():
                    wait_unit(bwq_v, sem_of(U_BWQ))
            off = pl.multiple_of(g * 1024 + t * 512, 512)
            q = _dot(x_v[...], bwq_v[:, pl.ds(off, 512)], NN)
            for e in range(4):
                head_rows(qb_s, g)[pl.ds(4 * t + e, B, stride=H), :] = (
                    q[:, e * 128:(e + 1) * 128])
    loop(4, bwq_step)

    def wuv_head(g, e, w):
        lat = jnp.concatenate(
            [head_rows(lat_s.at[ct], g)[pl.ds(e, B, stride=H), :]
             for ct in range(4)], axis=1).astype(BF16)
        r = pl.multiple_of(g * 64 + e * 8, 8)
        ctxa_s[pl.ds(r, 8), :] = _dot(lat, w, NN)
    weight_unit(wuv_v, U_WUV, lambda g, t: issue_kv(1, g, t, sem_of(U_KV + 1)), wuv_head)

    def kv_unit(b):
        u = U_KV + b

        def issue(g, t):
            sem = sem_of(u + 2)

            @pl.when(b < B - 2)
            def _():
                issue_kv(jnp.minimum(b + 2, B - 1), g, t, sem)

            @pl.when(b == B - 2)
            def _():
                issue_wide(wo_h, wo_v, 2 * g + t, sem)

            @pl.when(b == B - 1)
            def _():
                issue_bwo(2 * g + t)

        def pair_step(i):
            issue(i, 0)

            @pl.when(i == 0)
            def _():
                wait_unit(kv_v.at[b], sem_of(u))
            if "kv" in SKIP:
                issue(i, 1)
                return
            r = pl.multiple_of(b * H + i * 8, 8)
            q = qb_s[pl.ds(r, 8), :].astype(BF16)
            lo = lax.broadcasted_iota(jnp.int32, (8, W), 0) < 4
            s0 = _dot(q, kv_v[b, 0, 2 * i], NT)
            s1 = _dot(q, kv_v[b, 0, 2 * i + 1], NT)
            s = jnp.where(lo, s0, s1) * SCALE
            sb_s[...] = s - jnp.max(s, axis=1, keepdims=True)
            issue(i, 1)
            p = jnp.exp(sb_s[...])
            l = jnp.sum(p, axis=1, keepdims=True)
            pb = p.astype(BF16)
            o0 = _dot(pb, kv_v[b, 1, 2 * i], NN)
            o1 = _dot(pb, kv_v[b, 1, 2 * i + 1], NN)
            lo = lax.broadcasted_iota(jnp.int32, (8, D), 0) < 4
            o = jnp.where(lo, o0, o1) / l
            ctxb_s[pl.ds(r, 8), :] = o
        loop(4, pair_step)
    loop(B, kv_unit)

    x = x_v[...].astype(F32)
    gw = g_v[...].astype(F32).reshape(1, M)
    g = jax.nn.sigmoid(jnp.sum(x * gw, axis=1, keepdims=True))
    ctxa = jnp.concatenate(
        [ctxa_s[h * 8:(h + 1) * 8, :] for h in range(H)], axis=1).astype(BF16)
    ctxb = jnp.concatenate(
        [ctxb_s[pl.ds(h, B, stride=H), :] for h in range(H)], axis=1)
    rot = 32 + REM_BWO
    ctxb = jnp.concatenate([ctxb[:, rot:], ctxb[:, :rot]], axis=1).astype(BF16)

    def bwo_part(p, m):
        if "tail" in SKIP:
            return x
        lhs = jnp.concatenate(
            [ctxb[:, c:c + 128]
             for c in range(512 * p + 128 * m, H * D, 1024)], axis=1)
        return _dot(lhs, bwo_v[p, m], NN)

    if "waits" in SKIP:
        for u in range(20):
            wait_unit(wo_v, sem_of(u), True)
    wait_unit(wo_v, sem_of(U_WO), True)
    ga = g * _dot(ctxa, wo_v[...], NN)
    wait_unit(bwo_v.at[0], sem_of(U_BWO), True)
    bb = bwo_part(0, 0)
    for m in range(1, 4):
        bb = bb + bwo_part(0, m)
    for m in range(4):
        wait_unit(bwo_v.at[1, m], sems.at[NRING + m], True)
        bb = bb + bwo_part(1, m)
    o_ref[...] = (ga + (1.0 - g) * bb).astype(o_ref.dtype)


@jax.jit
def pallas_gated_mix__compressed_kv_cla__sliding_block_cached__decode_kernel(
    A_x: jax.Array,
    A_c_kv: jax.Array,
    A_w_q: jax.Array,
    A_w_uk: jax.Array,
    A_w_uv: jax.Array,
    A_w_o: jax.Array,
    B_x: jax.Array,
    B_k_cache: jax.Array,
    B_v_cache: jax.Array,
    B_wq: jax.Array,
    B_wo: jax.Array,
    gate_w: jax.Array,
):
    del B_x
    hbm = pl.BlockSpec(memory_space=pl.ANY)
    out = pl.pallas_call(
        _kernel,
        out_shape=jax.ShapeDtypeStruct((B, M), A_x.dtype),
        in_specs=[hbm] * 11,
        out_specs=pl.BlockSpec(memory_space=pltpu.VMEM),
        scratch_shapes=[
            pltpu.VMEM((B, M), BF16),
            pltpu.VMEM((M,), BF16),
            pltpu.VMEM((B, SK, C), BF16),
            pltpu.VMEM((M * H, D), BF16),
            pltpu.VMEM((C * H, D), BF16),
            pltpu.VMEM((C * H, D), BF16),
            pltpu.VMEM((H * D, M), BF16),
            pltpu.VMEM((B, 2, HKV, W, D), BF16),
            pltpu.VMEM((M, H * D), BF16),
            pltpu.VMEM((2, 4, 512, M), BF16),
            pltpu.VMEM((H * B, D), F32),
            pltpu.VMEM((4, H * B, 128), F32),
            pltpu.VMEM((4, H, SK // 4), F32),
            pltpu.VMEM((4, B * H, 128), F32),
            pltpu.VMEM((H * B, D), F32),
            pltpu.VMEM((H * B, D), F32),
            pltpu.VMEM((B * H, D), F32),
            pltpu.VMEM((8, W), F32),
            pltpu.SemaphoreType.DMA((NSEM,)),
        ],
        compiler_params=pltpu.CompilerParams(
            vmem_limit_bytes=100 * 1024 * 1024,
            disable_bounds_checks=True,
        ),
    )(
        A_x.reshape(B, M), A_c_kv,
        A_w_q.reshape(M * H, D), A_w_uk.reshape(C * H, D), A_w_uv.reshape(C * H, D),
        A_w_o.reshape(H * D, M), B_k_cache, B_v_cache, B_wq, B_wo, gate_w,
    )
    return out.reshape(B, 1, M)
```

```python
import jax
import jax.numpy as jnp
from jax import lax
import jax.experimental.pallas as pl
import jax.experimental.pallas.tpu as pltpu

B = 8
H = 32
D = 128
M = 512
C = 512
SK = 4096
HKV = 8
W = 1024
SCALE = D ** -0.5

NPIECE = 8
NRING = 4
NSEM = NRING + 4

REM_W = 8
REM_CKV = 0
REM_BWO = 8
REM_KV = 40
REM_BWQ = 5

PITCH = 24
KV_HEADS = (0, 1, 2, 3, 4, 5, 6, 7)
SPLIT = 2
PAT = (16, 64)
SKIP = ()
BENCH = None
F32 = jnp.float32
BF16 = jnp.bfloat16
U32 = jnp.uint32

NN = (((1,), (0,)), ((), ()))
NT = (((1,), (1,)), ((), ()))


def _dot(a, b, dims):
    return lax.dot_general(a, b, dims, preferred_element_type=F32)


def _kernel(x_h, ckv_h, wq_h, wuk_h, wuv_h, wo_h, k_h, v_h, bwq_h, bwo_h, g_h,
            o_ref,
            x_v, g_v, ckv_v, wq_v, wuk_v, wuv_v, wo_v, kv_v, bwq_v, bwo_v,
            wrl_s, qa_s, qabs_s, s_s, lat_s, qb_s, ctxa_s, ctxb_s, sb_s, sems):

    def chunk_bits(i):
        b1 = (i >> 1) & 1
        return (i & 1) * PAT[0] + b1 * 32 + ((i >> 2) & 1) * PAT[1] + (i >> 3), b1

    def copy(src, dst, sem, prio):
        pltpu.make_async_copy(src, dst, sem).start(priority=prio)

    def issue_rows(src, dst, nrows, rem, j, sem):
        rpc = nrows // 128
        align = 8 if rem else rpc
        jx = (j, j ^ 1)
        for i in range(16):
            hi, b1 = chunk_bits(i)
            start = (hi + 1) * rpc + rem + jx[b1] * (2 * rpc)
            if i == 15:
                start = jnp.where(j == 6, rem, start)
            sm = sem(i) if callable(sem) else sem

            def go(r, r0, n, i=i, b1=b1, sm=sm):
                d = dst(i, jx[b1], r0, n) if callable(dst) else dst.at[pl.ds(r, n)]
                copy(src.at[pl.ds(r, n)], d, sm, i % 2)

            if i == 7 and rem:
                @pl.when(j == 6)
                def _():
                    go(nrows - rpc + rem, 0, rpc - rem)
                    go(0, rpc - rem, rem)

                @pl.when(j != 6)
                def _():
                    go(pl.multiple_of(start, align), 0, rpc)
            else:
                go(pl.multiple_of(start, align), 0, rpc)

    def issue_bwq(j, sem):
        c0, c1 = REM_BWQ * 128, (REM_BWQ + 16) * 128
        jx = (j, j ^ 1)
        for i in range(16):
            hi, b1 = chunk_bits(i)
            r = pl.multiple_of((hi // 2) * 8 + jx[b1] * 8, 8)
            rn = pl.multiple_of((r + 8) & (M - 1), 8)

            def go(r, c, n, i=i):
                copy(bwq_h.at[pl.ds(r, 8), pl.ds(c, n)],
                     bwq_v.at[pl.ds(r, 8), pl.ds(c, n)], sem, i % 2)

            if i < 8:
                go(r, c1, H * D - c1)
                if c0:
                    go(rn, 0, c0)
            else:
                go(rn, c0, c1 - c0)

    def issue_kv(b, g, t, sem):
        def piece(edge):
            for h in KV_HEADS:
                k = (2 * g + t) ^ (2 * (h & 1))
                start = pl.multiple_of(((k + 1) * 128 + REM_KV) & (W - 1), 8)
                for a, src in enumerate((k_h, v_h)):
                    def go(r, n):
                        copy(src.at[b, h, pl.ds(SK - W + r, n)],
                             kv_v.at[b, a, h, pl.ds(r, n)], sem, a)
                    if edge != h & 1:
                        go(start, 128)
                    elif t == 0:
                        go(W - 128 + REM_KV, 128 - REM_KV)
                    else:
                        go(0, 128 + REM_KV)
        pl.when(g < 2)(lambda: piece(None))
        pl.when(g == 2)(lambda: piece(1))
        pl.when(g == 3)(lambda: piece(0))

    def issue_wide(src, dst, j, sem):
        if not SPLIT:
            return issue_rows(src, dst, 4096, REM_CKV, j, sem)
        jx = (j, j ^ 1)
        for i in range(16):
            hi, b1 = chunk_bits(i)
            r = (hi + 1) * 32 + jx[b1] * 64
            if i == 15:
                r = jnp.where(j == 6, 0, r)
            r = pl.multiple_of(r, 32)

            def go(r, n, c, m, i=i):
                copy(src.at[pl.ds(r, n), pl.ds(c, m)],
                     dst.at[pl.ds(r, n), pl.ds(c, m)], sem, i % 2)

            if SPLIT == 2:
                go(r, 32, 128, 384)
                if i in (7, 15):
                    pl.when(j == 6)(
                        (lambda: go(4096 - 24, 24, 0, 128)) if i == 7
                        else (lambda: go(0, 40, 0, 128)))
                    pl.when(j != 6)(lambda: go(r + 8, 32, 0, 128))
                else:
                    go(r + 8, 32, 0, 128)
            else:
                if i == 15:
                    pl.when(j == 6)(lambda: go(0, 8, 0, 128))
                go(r, 8, 128, 384)
                go(r + 8, 24, 0, 512)
                if i == 7:
                    pl.when(j != 6)(lambda: go(r + 32, 8, 0, 128))
                else:
                    go(r + 32, 8, 0, 128)

    def issue_ckv(b, j, sem):
        issue_wide(ckv_h.at[b], ckv_v.at[b], j, sem)

    def issue_bwo(j):
        def dst(i, jj, r0, n):
            s4 = ((i >> 1) & 1) + 2 * ((i >> 2) & 1)
            r = s4 * 128 + (i >> 3) * 32 + (jj & 1) * 64 + r0
            return bwo_v.at[i & 1, jj >> 1, pl.ds(pl.multiple_of(r, 8), n)]

        def sem(i):
            return sems.at[NRING + (j >> 1)] if i & 1 else sem_of(U_BWO)
        issue_rows(bwo_h, dst, H * D, REM_BWO, j, sem)

    def wait_unit(buf, sem, force=False):
        if "waits" in SKIP and not force:
            return
        pltpu.make_async_copy(buf, buf, sem).wait()

    def sem_of(u):
        return sems.at[u % NRING]

    def loop(n, body):
        def f(i, c):
            body(i)
            return c
        lax.fori_loop(0, n, f, 0)

    U_WQ, U_WUK, U_CKV, U_BWQ, U_WUV, U_KV, U_WO, U_BWO = 0, 1, 2, 10, 11, 12, 20, 21

    if BENCH is not None:
        sm = sems.at[0]
        n = 0
        for w in BENCH:
            if w in ("wq", "wuk", "wuv"):
                hh, vv = dict(wq=(wq_h, wq_v), wuk=(wuk_h, wuk_v), wuv=(wuv_h, wuv_v))[w]
                loop(8, lambda j: issue_rows(hh, vv, M * H, REM_W, j, sm)); n += 1
            elif w == "wo":
                loop(8, lambda j: issue_wide(wo_h, wo_v, j, sm)); n += 1
            elif w == "bwo":
                loop(8, lambda j: issue_rows(bwo_h, wo_v, H * D, REM_BWO, j, sm)); n += 1
            elif w == "bwq":
                loop(8, lambda j: issue_bwq(j, sm)); n += 1
            elif w == "ckv":
                loop(8, lambda b: loop(8, lambda j: issue_ckv(b, j, sm))); n += 8
            elif w == "kv":
                def f(b, g):
                    issue_kv(b, g, 0, sm)
                    issue_kv(b, g, 1, sm)
                loop(8, lambda b: loop(4, lambda g: f(b, g))); n += 8
        for _ in range(n):
            wait_unit(wo_v, sm, True)
        o_ref[...] = jnp.zeros_like(o_ref)
        return

    cx = pltpu.make_async_copy(x_h, x_v, sems.at[3])
    cg = pltpu.make_async_copy(g_h, g_v, sems.at[3])
    cx.start()
    cg.start()
    loop(NPIECE, lambda j: issue_rows(wq_h, wq_v, M * H, REM_W, j, sem_of(U_WQ)))
    loop(NPIECE, lambda j: issue_rows(wuk_h, wuk_v, C * H, REM_W, j, sem_of(U_WUK)))
    cx.wait()
    cg.wait()

    def relayout(w_v, q):
        def body(i, c):
            r = pl.multiple_of((q * 64 + i) * 64, 64)
            d = pl.multiple_of((q * 64 + i) * PITCH, 8)
            val = pltpu.bitcast(w_v[pl.ds(r, 64), :], U32)
            wrl_s[0, pl.ds(d, 16), :] = val[:16]
            wrl_s[1, pl.ds(d, 16), :] = val[16:]
            return c
        lax.fori_loop(0, 64, body, 0, unroll=8)

    def head_pair(g, t):
        rows = pl.ds(pl.multiple_of(8 * g, 8), 256 * PITCH - 8)
        a = wrl_s.at[0, rows][pl.ds(t, 256, stride=PITCH), :]
        b = wrl_s.at[1, rows][pl.ds(t, 256, stride=PITCH), :]
        w0 = pltpu.bitcast((a & U32(0xFFFF)) | (b << 16), BF16)
        w1 = pltpu.bitcast((a >> 16) | (b & U32(0xFFFF0000)), BF16)
        return w0, w1

    def head_rows(ref, h0, n):
        return ref.at[pl.ds(pl.multiple_of(h0, 8), B * H - H + n)]

    def weight_unit(w_v, u, issue, per_head):
        def step1(g):
            for t in range(2):
                issue(g, t)
                if t == 0:
                    @pl.when(g == 0)
                    def _():
                        wait_unit(w_v, sem_of(u))
                if "w" not in SKIP:
                    relayout(w_v, 2 * g + t)
        loop(2, step1)

        def step2(g):
            for t in range(8):
                if t % 4 == 0:
                    issue(2 + g, t // 4)
                if "w" in SKIP:
                    continue
                ws = head_pair(g, t)
                per_head(g, 2 * t, ws[0])
                per_head(g, 2 * t + 1, ws[1])
        loop(2, step2)

    def wq_head(g, e, w):
        r = pl.multiple_of(g * 128 + e * 8, 8)
        qa_s[pl.ds(r, 8), :] = _dot(x_v[...], w, NN)
    weight_unit(wq_v, U_WQ, lambda g, t: issue_ckv(0, 2 * g + t, sem_of(U_CKV)), wq_head)

    def wuk_head(g, e, w):
        r = pl.multiple_of(g * 128 + e * 8, 8)
        q = qa_s[pl.ds(r, 8), :].astype(BF16)
        qa = _dot(q, w, NT) * SCALE
        for ct in range(4):
            head_rows(qabs_s.at[ct], 16 * g, 16)[pl.ds(e, B, stride=H), :] = (
                qa[:, ct * 128:(ct + 1) * 128])
    weight_unit(wuk_v, U_WUK, lambda g, t: issue_ckv(1, 2 * g + t, sem_of(U_CKV + 1)), wuk_head)

    def ckv_unit(b):
        u = U_CKV + b

        def issue(j):
            sem = sem_of(u + 2)

            @pl.when(b < B - 2)
            def _():
                issue_ckv(jnp.minimum(b + 2, B - 1), j, sem)

            @pl.when(b == B - 2)
            def _():
                issue_bwq(j, sem)

            @pl.when(b == B - 1)
            def _():
                issue_rows(wuv_h, wuv_v, C * H, REM_W, j, sem)

        issue(0)
        wait_unit(ckv_v.at[b], sem_of(u))
        r = pl.multiple_of(b * H, H)
        qa = jnp.concatenate(
            [qabs_s[ct, pl.ds(r, H), :] for ct in range(4)], axis=1
        ).astype(BF16)
        KC = SK // 4

        def score_step(j, m):
            @pl.when(j > 0)
            def _():
                issue(j)
            if "ckv" in SKIP:
                return m
            off = pl.multiple_of(j * KC, KC)
            s = _dot(qa, ckv_v[b, pl.ds(off, KC), :], NT)
            s_s[j] = s
            for t in range(KC // 128):
                m = jnp.maximum(m, s[:, t * 128:(t + 1) * 128])
            return m
        m = lax.fori_loop(0, 4, score_step, jnp.full((H, 128), -jnp.inf, F32))
        m = jnp.max(m, axis=1, keepdims=True)

        def pv_step(j, carry):
            l, acc = carry
            issue(4 + j)
            if "ckv" in SKIP:
                return l + s_s[j][:, :128], acc + s_s[j][:, :512]
            off = pl.multiple_of(j * KC, KC)
            p = jnp.exp(s_s[j] - m)
            for t in range(KC // 128):
                l = l + p[:, t * 128:(t + 1) * 128]
            acc = acc + _dot(p.astype(BF16), ckv_v[b, pl.ds(off, KC), :], NN)
            return l, acc
        l, acc = lax.fori_loop(
            0, 4, pv_step, (jnp.zeros((H, 128), F32), jnp.zeros((H, C), F32)))
        lat = acc / jnp.sum(l, axis=1, keepdims=True)
        for ct in range(4):
            lat_s[ct, pl.ds(r, H), :] = lat[:, ct * 128:(ct + 1) * 128]
    loop(B, ckv_unit)

    def bwq_step(g):
        for t in range(2):
            issue_kv(0, g, t, sem_of(U_KV))
            if t == 0:
                @pl.when(g == 0)
                def _():
                    wait_unit(bwq_v, sem_of(U_BWQ))
            off = pl.multiple_of(g * 1024 + t * 512, 512)
            q = _dot(x_v[...], bwq_v[:, pl.ds(off, 512)], NN)
            for e in range(4):
                head_rows(qb_s, 8 * g, 8)[pl.ds(4 * t + e, B, stride=H), :] = (
                    q[:, e * 128:(e + 1) * 128])
    loop(4, bwq_step)

    def wuv_head(g, e, w):
        lat = jnp.concatenate(
            [head_rows(lat_s.at[ct], 16 * g, 16)[pl.ds(e, B, stride=H), :]
             for ct in range(4)], axis=1).astype(BF16)
        r = pl.multiple_of(g * 128 + e * 8, 8)
        ctxa_s[pl.ds(r, 8), :] = _dot(lat, w, NN)
    weight_unit(wuv_v, U_WUV, lambda g, t: issue_kv(1, g, t, sem_of(U_KV + 1)), wuv_head)

    def kv_unit(b):
        u = U_KV + b

        def issue(g, t):
            sem = sem_of(u + 2)

            @pl.when(b < B - 2)
            def _():
                issue_kv(jnp.minimum(b + 2, B - 1), g, t, sem)

            @pl.when(b == B - 2)
            def _():
                issue_wide(wo_h, wo_v, 2 * g + t, sem)

            @pl.when(b == B - 1)
            def _():
                issue_bwo(2 * g + t)

        def pair_step(i):
            issue(i, 0)

            @pl.when(i == 0)
            def _():
                wait_unit(kv_v.at[b], sem_of(u))
            if "kv" in SKIP:
                issue(i, 1)
                return
            r = pl.multiple_of(b * H + i * 8, 8)
            q = qb_s[pl.ds(r, 8), :].astype(BF16)
            lo = lax.broadcasted_iota(jnp.int32, (8, W), 0) < 4
            s0 = _dot(q, kv_v[b, 0, 2 * i], NT)
            s1 = _dot(q, kv_v[b, 0, 2 * i + 1], NT)
            s = jnp.where(lo, s0, s1) * SCALE
            sb_s[...] = s - jnp.max(s, axis=1, keepdims=True)
            issue(i, 1)
            p = jnp.exp(sb_s[...])
            l = jnp.sum(p, axis=1, keepdims=True)
            pb = p.astype(BF16)
            o0 = _dot(pb, kv_v[b, 1, 2 * i], NN)
            o1 = _dot(pb, kv_v[b, 1, 2 * i + 1], NN)
            lo = lax.broadcasted_iota(jnp.int32, (8, D), 0) < 4
            o = jnp.where(lo, o0, o1) / l
            ctxb_s[pl.ds(r, 8), :] = o
        loop(4, pair_step)
    loop(B, kv_unit)

    x = x_v[...].astype(F32)
    gw = g_v[...].astype(F32).reshape(1, M)
    g = jax.nn.sigmoid(jnp.sum(x * gw, axis=1, keepdims=True))
    ctxa = jnp.concatenate(
        [ctxa_s[h * 8:(h + 1) * 8, :] for h in range(H)], axis=1).astype(BF16)
    ctxb = jnp.concatenate(
        [ctxb_s[pl.ds(h, B, stride=H), :] for h in range(H)], axis=1)
    rot = 32 + REM_BWO
    ctxb = jnp.concatenate([ctxb[:, rot:], ctxb[:, :rot]], axis=1).astype(BF16)

    def bwo_part(p, m):
        if "tail" in SKIP:
            return x
        lhs = jnp.concatenate(
            [ctxb[:, c:c + 128]
             for c in range(512 * p + 128 * m, H * D, 1024)], axis=1)
        return _dot(lhs, bwo_v[p, m], NN)

    if "waits" in SKIP:
        for u in range(20):
            wait_unit(wo_v, sem_of(u), True)
    wait_unit(wo_v, sem_of(U_WO), True)
    ga = g * _dot(ctxa, wo_v[...], NN)
    wait_unit(bwo_v.at[0], sem_of(U_BWO), True)
    bb = bwo_part(0, 0)
    for m in range(1, 4):
        bb = bb + bwo_part(0, m)
    for m in range(4):
        wait_unit(bwo_v.at[1, m], sems.at[NRING + m], True)
        bb = bb + bwo_part(1, m)
    o_ref[...] = (ga + (1.0 - g) * bb).astype(o_ref.dtype)


@jax.jit
def pallas_gated_mix__compressed_kv_cla__sliding_block_cached__decode_kernel(
    A_x: jax.Array,
    A_c_kv: jax.Array,
    A_w_q: jax.Array,
    A_w_uk: jax.Array,
    A_w_uv: jax.Array,
    A_w_o: jax.Array,
    B_x: jax.Array,
    B_k_cache: jax.Array,
    B_v_cache: jax.Array,
    B_wq: jax.Array,
    B_wo: jax.Array,
    gate_w: jax.Array,
):
    del B_x
    hbm = pl.BlockSpec(memory_space=pl.ANY)
    out = pl.pallas_call(
        _kernel,
        out_shape=jax.ShapeDtypeStruct((B, M), A_x.dtype),
        in_specs=[hbm] * 11,
        out_specs=pl.BlockSpec(memory_space=pltpu.VMEM),
        scratch_shapes=[
            pltpu.VMEM((B, M), BF16),
            pltpu.VMEM((M,), BF16),
            pltpu.VMEM((B, SK, C), BF16),
            pltpu.VMEM((M * H, D), BF16),
            pltpu.VMEM((C * H, D), BF16),
            pltpu.VMEM((C * H, D), BF16),
            pltpu.VMEM((H * D, M), BF16),
            pltpu.VMEM((B, 2, HKV, W, D), BF16),
            pltpu.VMEM((M, H * D), BF16),
            pltpu.VMEM((2, 4, 512, M), BF16),
            pltpu.VMEM((2, 256 * PITCH, D), U32),
            pltpu.VMEM((H * B, D), F32),
            pltpu.VMEM((4, H * B, 128), F32),
            pltpu.VMEM((4, H, SK // 4), F32),
            pltpu.VMEM((4, B * H, 128), F32),
            pltpu.VMEM((H * B, D), F32),
            pltpu.VMEM((H * B, D), F32),
            pltpu.VMEM((B * H, D), F32),
            pltpu.VMEM((8, W), F32),
            pltpu.SemaphoreType.DMA((NSEM,)),
        ],
        compiler_params=pltpu.CompilerParams(
            vmem_limit_bytes=110 * 1024 * 1024,
            disable_bounds_checks=True,
        ),
    )(
        A_x.reshape(B, M), A_c_kv,
        A_w_q.reshape(M * H, D), A_w_uk.reshape(C * H, D), A_w_uv.reshape(C * H, D),
        A_w_o.reshape(H * D, M), B_k_cache, B_v_cache, B_wq, B_wo, gate_w,
    )
    return out.reshape(B, 1, M)
```

```python
import jax
import jax.numpy as jnp
from jax import lax
import jax.experimental.pallas as pl
import jax.experimental.pallas.tpu as pltpu

B = 8
H = 32
D = 128
M = 512
C = 512
SK = 4096
HKV = 8
W = 1024
SCALE = D ** -0.5

NPIECE = 8
NRING = 4

BWO_GROUPS = (
    [m + 8 * s for m in (0, 1, 2, 4) for s in range(4)],
    [m + 8 * s for m in (3, 5) for s in range(4)],
    [6 + 8 * s for s in range(4)],
    [7, 15], [23], [31],
)
BWO_LAST = (28, 62, 29, 63, 30, 60, 31, 61, 92, 93, 94, 95, 124, 125, 126, 127)
BWO_POS = {q: k for k, q in enumerate(sum(BWO_GROUPS, []))}
NSEM = NRING + len(BWO_GROUPS)

REM_W = 8
REM_CKV = 0
REM_BWO = 8
REM_KV = 40
REM_BWQ = 5

BWO_ROT = 32 + REM_BWO
CB_PITCH = 40
PITCH = 24
KV_HEADS = (0, 1, 2, 3, 4, 5, 6, 7)
SPLIT = 2
PAT = (16, 64)
PREFILL = 2
NOSEMCHK = True
SKIP = ()
BENCH = None
F32 = jnp.float32
BF16 = jnp.bfloat16
U32 = jnp.uint32

NN = (((1,), (0,)), ((), ()))
NT = (((1,), (1,)), ((), ()))


def _dot(a, b, dims):
    return lax.dot_general(a, b, dims, preferred_element_type=F32)


def _kernel(x_h, ckv_h, wq_h, wuk_h, wuv_h, wo_h, k_h, v_h, bwq_h, bwo_h, g_h,
            o_ref,
            x_v, g_v, ckv_v, wq_v, wuk_v, wuv_v, kv_v, bwq_v, wob_v,
            wrl_s, qa_s, qabs_s, s_s, lat_s, qb_s, ctx_s, ctxb_s, sb_s, gate_s, sems):
    wo_v = wob_v.at[pl.ds(0, H * D)]
    bwo_v = wob_v.at[pl.ds(H * D, H * D)]

    def chunk_bits(i):
        b1 = (i >> 1) & 1
        return (i & 1) * PAT[0] + b1 * 32 + ((i >> 2) & 1) * PAT[1] + (i >> 3), b1

    def copy(src, dst, sem, prio):
        pltpu.make_async_copy(src, dst, sem).start(priority=prio)

    def issue_rows(src, dst, nrows, rem, j, sem, prio=None):
        rpc = nrows // 128
        align = 8 if rem else rpc
        jx = (j, j ^ 1)
        order = range(16) if prio is None else [*range(0, 16, 2), *range(1, 16, 2)]
        for i in order:
            hi, b1 = chunk_bits(i)
            start = (hi + 1) * rpc + rem + jx[b1] * (2 * rpc)
            if i == 15:
                start = jnp.where(j == 6, rem, start)
            sm = sem(i) if callable(sem) else sem

            def go(r, r0, n, i=i, b1=b1, sm=sm):
                d = dst(i, jx[b1], r0, n) if callable(dst) else dst.at[pl.ds(r, n)]
                copy(src.at[pl.ds(r, n)], d, sm, i % 2 if prio is None else prio)

            if i == 7 and rem:
                @pl.when(j == 6)
                def _():
                    go(nrows - rpc + rem, 0, rpc - rem)
                    go(0, rpc - rem, rem)

                @pl.when(j != 6)
                def _():
                    go(pl.multiple_of(start, align), 0, rpc)
            else:
                go(pl.multiple_of(start, align), 0, rpc)

    def issue_bwq(j, sem):
        c0, c1 = REM_BWQ * 128, (REM_BWQ + 16) * 128
        jx = (j, j ^ 1)
        for i in range(16):
            hi, b1 = chunk_bits(i)
            r = pl.multiple_of((hi // 2) * 8 + jx[b1] * 8, 8)
            rn = pl.multiple_of((r + 8) & (M - 1), 8)

            def go(r, c, n, i=i):
                copy(bwq_h.at[pl.ds(r, 8), pl.ds(c, n)],
                     bwq_v.at[pl.ds(r, 8), pl.ds(c, n)], sem, i % 2)

            if i < 8:
                go(r, c1, H * D - c1)
                if c0:
                    go(rn, 0, c0)
            else:
                go(rn, c0, c1 - c0)

    def issue_kv(b, g, t, sem):
        def piece(edge):
            for h in KV_HEADS:
                k = (2 * g + t) ^ (2 * (h & 1))
                start = pl.multiple_of(((k + 1) * 128 + REM_KV) & (W - 1), 8)
                for a, src in enumerate((k_h, v_h)):
                    def go(r, n):
                        copy(src.at[b, h, pl.ds(SK - W + r, n)],
                             kv_v.at[b, a, h, pl.ds(r, n)], sem, a)
                    if edge != h & 1:
                        go(start, 128)
                    elif t == 0:
                        go(W - 128 + REM_KV, 128 - REM_KV)
                    else:
                        go(0, 128 + REM_KV)
        pl.when(g < 2)(lambda: piece(None))
        pl.when(g == 2)(lambda: piece(1))
        pl.when(g == 3)(lambda: piece(0))

    def issue_wide(src, dst, j, sem):
        if not SPLIT:
            return issue_rows(src, dst, 4096, REM_CKV, j, sem)
        jx = (j, j ^ 1)
        for i in range(16):
            hi, b1 = chunk_bits(i)
            r = (hi + 1) * 32 + jx[b1] * 64
            if i == 15:
                r = jnp.where(j == 6, 0, r)
            r = pl.multiple_of(r, 32)

            def go(r, n, c, m, i=i):
                copy(src.at[pl.ds(r, n), pl.ds(c, m)],
                     dst.at[pl.ds(r, n), pl.ds(c, m)], sem, i % 2)

            if SPLIT == 2:
                go(r, 32, 128, 384)
                if i in (7, 15):
                    pl.when(j == 6)(
                        (lambda: go(4096 - 24, 24, 0, 128)) if i == 7
                        else (lambda: go(0, 40, 0, 128)))
                    pl.when(j != 6)(lambda: go(r + 8, 32, 0, 128))
                else:
                    go(r + 8, 32, 0, 128)
            else:
                if i == 15:
                    pl.when(j == 6)(lambda: go(0, 8, 0, 128))
                go(r, 8, 128, 384)
                go(r + 8, 24, 0, 512)
                if i == 7:
                    pl.when(j != 6)(lambda: go(r + 32, 8, 0, 128))
                else:
                    go(r + 32, 8, 0, 128)

    def issue_ckv(b, j, sem):
        issue_wide(ckv_h.at[b], ckv_v.at[b], j, sem)

    def bwo_sem(grp):
        return sems.at[NRING + grp]

    def issue_bwo(g, t):
        @pl.when(g < 3)
        def _():
            j = 2 * g + t
            jx = (j, j ^ 1)
            shift = (4 * g, jnp.where(g == 0, 0, 4 + 4 * g))
            for i in range(16):
                hi, b1 = chunk_bits(i)
                r = (hi + 1) * 32 + REM_BWO + jx[b1] * 64
                d = (BWO_POS[hi // 4] + shift[i & 1]) * 128 + (hi % 4 + 2 * (t ^ b1)) * 32
                copy(bwo_h.at[pl.ds(pl.multiple_of(r, 8), 32)],
                     bwo_v.at[pl.ds(pl.multiple_of(d, 32), 32)],
                     bwo_sem(g if i & 1 else 0), i & 1)

        @pl.when(g == 3)
        def _():
            for i in range(16):
                hi, b1 = chunk_bits(i)
                u = hi + 2 * ((6 + t) ^ b1) if i % 2 == 0 else BWO_LAST[8 * t + i // 2]
                grp = next(k for k, qs in enumerate(BWO_GROUPS) if u // 4 in qs)
                r = (u + 1) * 32 + REM_BWO
                d = BWO_POS[u // 4] * 128 + (u % 4) * 32
                n = min(32, H * D - r) if r < H * D else 32
                for r0, nn in ((0, n), (n, 32 - n)):
                    if nn:
                        copy(bwo_h.at[pl.ds((r + r0) % (H * D), nn)],
                             bwo_v.at[pl.ds(d + r0, nn)], bwo_sem(grp), i & 1)

    def wait_unit(buf, sem, force=False):
        if "waits" in SKIP and not force:
            return
        pltpu.make_async_copy(buf, buf, sem).wait()

    def sem_of(u):
        return sems.at[u % NRING]

    def loop(n, body):
        def f(i, c):
            body(i)
            return c
        lax.fori_loop(0, n, f, 0)

    U_WQ, U_WUK, U_CKV, U_BWQ, U_WUV, U_KV, U_WO, U_BWO = 0, 1, 2, 10, 11, 12, 20, 21

    if BENCH is not None:
        sm = sems.at[0]
        n = 0
        for w in BENCH:
            if w in ("wq", "wuk", "wuv"):
                hh, vv = dict(wq=(wq_h, wq_v), wuk=(wuk_h, wuk_v), wuv=(wuv_h, wuv_v))[w]
                loop(8, lambda j: issue_rows(hh, vv, M * H, REM_W, j, sm)); n += 1
            elif w == "wo":
                loop(8, lambda j: issue_wide(wo_h, wo_v, j, sm)); n += 1
            elif w == "bwo":
                loop(8, lambda j: issue_rows(bwo_h, wo_v, H * D, REM_BWO, j, sm)); n += 1
            elif w == "bwq":
                loop(8, lambda j: issue_bwq(j, sm)); n += 1
            elif w == "ckv":
                loop(8, lambda b: loop(8, lambda j: issue_ckv(b, j, sm))); n += 8
            elif w == "kv":
                def f(b, g):
                    issue_kv(b, g, 0, sm)
                    issue_kv(b, g, 1, sm)
                loop(8, lambda b: loop(4, lambda g: f(b, g))); n += 8
        for _ in range(n):
            wait_unit(wo_v, sm, True)
        o_ref[...] = jnp.zeros_like(o_ref)
        return

    cx = pltpu.make_async_copy(x_h, x_v, sems.at[3])
    cg = pltpu.make_async_copy(g_h, g_v, sems.at[3])
    cx.start()
    cg.start()
    loop(PREFILL, lambda j: issue_rows(wq_h, wq_v, M * H, REM_W, j, sem_of(U_WQ), 1))
    loop(NPIECE - PREFILL,
         lambda j: issue_rows(wq_h, wq_v, M * H, REM_W, j + PREFILL, sem_of(U_WQ)))
    loop(NPIECE, lambda j: issue_rows(wuk_h, wuk_v, C * H, REM_W, j, sem_of(U_WUK)))
    cx.wait()
    cg.wait()
    gate = jax.nn.sigmoid(jnp.sum(
        x_v[...].astype(F32) * g_v[...].astype(F32).reshape(1, M),
        axis=1, keepdims=True))
    gate_s[0] = jnp.broadcast_to(gate, (B, M))
    gate_s[1] = jnp.broadcast_to(1.0 - gate, (B, M))

    def relayout(w_v, q):
        def body(i, c):
            r = pl.multiple_of((q * 64 + i) * 64, 64)
            d = pl.multiple_of((q * 64 + i) * PITCH, 8)
            val = pltpu.bitcast(w_v[pl.ds(r, 64), :], U32)
            wrl_s[0, pl.ds(d, 16), :] = val[:16]
            wrl_s[1, pl.ds(d, 16), :] = val[16:]
            return c
        lax.fori_loop(0, 64, body, 0, unroll=8)

    def head_pair(g, t):
        rows = pl.ds(pl.multiple_of(8 * g, 8), 256 * PITCH - 8)
        a = wrl_s.at[0, rows][pl.ds(t, 256, stride=PITCH), :]
        b = wrl_s.at[1, rows][pl.ds(t, 256, stride=PITCH), :]
        w0 = pltpu.bitcast((a & U32(0xFFFF)) | (b << 16), BF16)
        w1 = pltpu.bitcast((a >> 16) | (b & U32(0xFFFF0000)), BF16)
        return w0, w1

    def head_rows(ref, h0, n):
        return ref.at[pl.ds(pl.multiple_of(h0, 8), B * H - H + n)]

    def weight_unit(w_v, u, issue, per_head):
        def step1(g):
            for t in range(2):
                issue(g, t)
                if t == 0:
                    @pl.when(g == 0)
                    def _():
                        wait_unit(w_v, sem_of(u))
                if "w" not in SKIP:
                    relayout(w_v, 2 * g + t)
        loop(2, step1)

        def step2(g):
            for t in range(8):
                if t % 4 == 0:
                    issue(2 + g, t // 4)
                if "w" in SKIP:
                    continue
                ws = head_pair(g, t)
                per_head(g, 2 * t, ws[0])
                per_head(g, 2 * t + 1, ws[1])
        loop(2, step2)

    def wq_head(g, e, w):
        r = pl.multiple_of(g * 128 + e * 8, 8)
        qa_s[pl.ds(r, 8), :] = _dot(x_v[...], w, NN)
    weight_unit(wq_v, U_WQ, lambda g, t: issue_ckv(0, 2 * g + t, sem_of(U_CKV)), wq_head)

    def wuk_head(g, e, w):
        r = pl.multiple_of(g * 128 + e * 8, 8)
        q = qa_s[pl.ds(r, 8), :].astype(BF16)
        qa = _dot(q, w, NT) * SCALE
        for ct in range(4):
            head_rows(qabs_s.at[ct], 16 * g, 16)[pl.ds(e, B, stride=H), :] = (
                qa[:, ct * 128:(ct + 1) * 128])
    weight_unit(wuk_v, U_WUK, lambda g, t: issue_ckv(1, 2 * g + t, sem_of(U_CKV + 1)), wuk_head)

    def ckv_unit(b):
        u = U_CKV + b

        def issue(j):
            sem = sem_of(u + 2)

            @pl.when(b < B - 2)
            def _():
                issue_ckv(jnp.minimum(b + 2, B - 1), j, sem)

            @pl.when(b == B - 2)
            def _():
                issue_bwq(j, sem)

            @pl.when(b == B - 1)
            def _():
                issue_rows(wuv_h, wuv_v, C * H, REM_W, j, sem)

        issue(0)
        wait_unit(ckv_v.at[b], sem_of(u))
        r = pl.multiple_of(b * H, H)
        qa = jnp.concatenate(
            [qabs_s[ct, pl.ds(r, H), :] for ct in range(4)], axis=1
        ).astype(BF16)
        KC = SK // 4

        def score_step(j, m):
            @pl.when(j > 0)
            def _():
                issue(j)
            if "ckv" in SKIP:
                return m
            off = pl.multiple_of(j * KC, KC)
            s = _dot(qa, ckv_v[b, pl.ds(off, KC), :], NT)
            s_s[j] = s
            for t in range(KC // 128):
                m = jnp.maximum(m, s[:, t * 128:(t + 1) * 128])
            return m
        m = lax.fori_loop(0, 4, score_step, jnp.full((H, 128), -jnp.inf, F32))
        m = jnp.max(m, axis=1, keepdims=True)

        def pv_step(j, carry):
            l, acc = carry
            issue(4 + j)
            if "ckv" in SKIP:
                return l + s_s[j][:, :128], acc + s_s[j][:, :512]
            off = pl.multiple_of(j * KC, KC)
            p = jnp.exp(s_s[j] - m)
            for t in range(KC // 128):
                l = l + p[:, t * 128:(t + 1) * 128]
            acc = acc + _dot(p.astype(BF16), ckv_v[b, pl.ds(off, KC), :], NN)
            return l, acc
        l, acc = lax.fori_loop(
            0, 4, pv_step, (jnp.zeros((H, 128), F32), jnp.zeros((H, C), F32)))
        lat = acc / jnp.sum(l, axis=1, keepdims=True)
        for ct in range(4):
            lat_s[ct, pl.ds(r, H), :] = lat[:, ct * 128:(ct + 1) * 128]
    loop(B, ckv_unit)

    def bwq_step(g):
        for t in range(2):
            issue_kv(0, g, t, sem_of(U_KV))
            if t == 0:
                @pl.when(g == 0)
                def _():
                    wait_unit(bwq_v, sem_of(U_BWQ))
            off = pl.multiple_of(g * 1024 + t * 512, 512)
            q = _dot(x_v[...], bwq_v[:, pl.ds(off, 512)], NN)
            for e in range(4):
                head_rows(qb_s, 8 * g, 8)[pl.ds(4 * t + e, B, stride=H), :] = (
                    q[:, e * 128:(e + 1) * 128])
    loop(4, bwq_step)

    def wuv_head(g, e, w):
        lat = jnp.concatenate(
            [head_rows(lat_s.at[ct], 16 * g, 16)[pl.ds(e, B, stride=H), :]
             for ct in range(4)], axis=1).astype(BF16)
        r = pl.multiple_of(g * 128 + e * 8, 8)
        ctx_s[pl.ds(r, 8), :] = _dot(lat, w, NN)
    weight_unit(wuv_v, U_WUV, lambda g, t: issue_kv(1, g, t, sem_of(U_KV + 1)), wuv_head)

    def kv_unit(b):
        u = U_KV + b

        def issue(g, t):
            sem = sem_of(u + 2)

            @pl.when(b < B - 2)
            def _():
                issue_kv(jnp.minimum(b + 2, B - 1), g, t, sem)

            @pl.when(b == B - 2)
            def _():
                issue_wide(wo_h, wo_v, 2 * g + t, sem)

            @pl.when(b == B - 1)
            def _():
                issue_bwo(g, t)

        def pair_step(i):
            issue(i, 0)

            @pl.when(i == 0)
            def _():
                wait_unit(kv_v.at[b], sem_of(u))
            if "kv" in SKIP:
                issue(i, 1)
                return
            r = pl.multiple_of(b * H + i * 8, 8)
            q = qb_s[pl.ds(r, 8), :].astype(BF16)
            lo = lax.broadcasted_iota(jnp.int32, (8, W), 0) < 4
            s0 = _dot(q, kv_v[b, 0, 2 * i], NT)
            s1 = _dot(q, kv_v[b, 0, 2 * i + 1], NT)
            s = jnp.where(lo, s0, s1) * SCALE
            sb_s[...] = s - jnp.max(s, axis=1, keepdims=True)
            issue(i, 1)
            p = jnp.exp(sb_s[...])
            l = jnp.sum(p, axis=1, keepdims=True)
            pb = p.astype(BF16)
            o0 = _dot(pb, kv_v[b, 1, 2 * i], NN)
            o1 = _dot(pb, kv_v[b, 1, 2 * i + 1], NN)
            lo = lax.broadcasted_iota(jnp.int32, (8, D), 0) < 4
            o = jnp.where(lo, o0, o1) / l
            rb = pl.multiple_of(b * CB_PITCH + i * 8, 8)
            ctxb_s[pl.ds(rb, 8), :] = pltpu.roll(o, D - BWO_ROT, 1)
        loop(4, pair_step)
    loop(B, kv_unit)

    lo = lax.broadcasted_iota(jnp.int32, (B, D), 1) < D - BWO_ROT
    heads = [ctxb_s[pl.ds(h, B, stride=CB_PITCH), :] for h in range(H)]
    for q in range(H):
        ctx_s[pl.ds((H + BWO_POS[q]) * 8, 8), :] = (
            jnp.where(lo, heads[q], heads[(q + 1) % H]))

    def proj(blk, n):
        r = blk * 8 if isinstance(blk, int) else pl.multiple_of(blk * 8, 8)
        lhs = jnp.concatenate(
            [ctx_s[pl.ds(r + 8 * k, 8), :] for k in range(n)], axis=1).astype(BF16)
        w = blk * 128 if isinstance(blk, int) else pl.multiple_of(blk * 128, 128)
        return _dot(lhs, wob_v[pl.ds(w, n * 128), :], NN)

    def wait_bwo(grp):
        qs = BWO_GROUPS[grp]
        rows = pl.ds(BWO_POS[qs[0]] * 128, len(qs) * 128)
        wait_unit(bwo_v.at[rows], bwo_sem(grp), True)

    if "waits" in SKIP:
        for u in range(20):
            wait_unit(wo_v, sem_of(u), True)

    def proj_step(it, acc):
        pl.when(it == 0)(lambda: wait_unit(wo_v, sem_of(U_WO), True))
        pl.when(it == 4)(lambda: wait_bwo(0))
        pl.when(it == 6)(lambda: wait_bwo(1))
        return acc + gate_s[it >> 2] * proj(8 * it, 8)
    acc = lax.fori_loop(0, 7, proj_step, jnp.zeros((B, M), F32))
    for grp in range(2, len(BWO_GROUPS)):
        wait_bwo(grp)
        if "tail" in SKIP:
            continue
        qs = BWO_GROUPS[grp]
        acc = acc + gate_s[1] * proj(H + BWO_POS[qs[0]], len(qs))
    o_ref[...] = acc.astype(o_ref.dtype)


@jax.jit
def pallas_gated_mix__compressed_kv_cla__sliding_block_cached__decode_kernel(
    A_x: jax.Array,
    A_c_kv: jax.Array,
    A_w_q: jax.Array,
    A_w_uk: jax.Array,
    A_w_uv: jax.Array,
    A_w_o: jax.Array,
    B_x: jax.Array,
    B_k_cache: jax.Array,
    B_v_cache: jax.Array,
    B_wq: jax.Array,
    B_wo: jax.Array,
    gate_w: jax.Array,
):
    del B_x
    hbm = pl.BlockSpec(memory_space=pl.ANY)
    out = pl.pallas_call(
        _kernel,
        out_shape=jax.ShapeDtypeStruct((B, M), A_x.dtype),
        in_specs=[hbm] * 11,
        out_specs=pl.BlockSpec(memory_space=pltpu.VMEM),
        scratch_shapes=[
            pltpu.VMEM((B, M), BF16),
            pltpu.VMEM((M,), BF16),
            pltpu.VMEM((B, SK, C), BF16),
            pltpu.VMEM((M * H, D), BF16),
            pltpu.VMEM((C * H, D), BF16),
            pltpu.VMEM((C * H, D), BF16),
            pltpu.VMEM((B, 2, HKV, W, D), BF16),
            pltpu.VMEM((M, H * D), BF16),
            pltpu.VMEM((2 * H * D, M), BF16),
            pltpu.VMEM((2, 256 * PITCH, D), U32),
            pltpu.VMEM((H * B, D), F32),
            pltpu.VMEM((4, H * B, 128), F32),
            pltpu.VMEM((4, H, SK // 4), F32),
            pltpu.VMEM((4, B * H, 128), F32),
            pltpu.VMEM((H * B, D), F32),
            pltpu.VMEM((2 * H * B, D), F32),
            pltpu.VMEM((B * CB_PITCH, D), F32),
            pltpu.VMEM((8, W), F32),
            pltpu.VMEM((2, B, M), F32),
            pltpu.SemaphoreType.DMA((NSEM,)),
        ],
        compiler_params=pltpu.CompilerParams(
            vmem_limit_bytes=110 * 1024 * 1024,
            disable_bounds_checks=True,
            disable_semaphore_checks=NOSEMCHK,
        ),
    )(
        A_x.reshape(B, M), A_c_kv,
        A_w_q.reshape(M * H, D), A_w_uk.reshape(C * H, D), A_w_uv.reshape(C * H, D),
        A_w_o.reshape(H * D, M), B_k_cache, B_v_cache, B_wq, B_wo, gate_w,
    )
    return out.reshape(B, 1, M)
```

```python
import jax
import jax.numpy as jnp
from jax import lax
import jax.experimental.pallas as pl
import jax.experimental.pallas.tpu as pltpu

B = 8
H = 32
D = 128
M = 512
C = 512
SK = 4096
HKV = 8
W = 1024
SCALE = D ** -0.5

F32 = jnp.float32
BF16 = jnp.bfloat16
U32 = jnp.uint32
NN = (((1,), (0,)), ((), ()))
NT = (((1,), (1,)), ((), ()))

U_WQ, U_WUK, U_CKV, U_BWQ, U_WUV, U_KV, U_WO = 0, 1, 2, 10, 11, 12, 20
NRING = 4
PREFILL = 2

REM_W = 8
REM_KV = 40
REM_BWO = 8
REM_BWQ = 5

W_PITCH = 24
CB_PITCH = 40
BWO_ROT = 32 + REM_BWO


def _chunk_bits(i):
    b1 = (i >> 1) & 1
    return (i & 1) * 64 + b1 * 32 + ((i >> 2) & 1) + (i >> 3) * 16, b1


def _bwo_tables():
    def blocks(prio, m):
        return [q + 16 * prio for q in range(m, 16, 4)]
    groups = (blocks(0, 0) + blocks(0, 1) + blocks(0, 2) + blocks(1, 0),
              blocks(0, 3) + blocks(1, 1), blocks(1, 2), [19, 27], [23], [31])
    pos = {q: k for k, q in enumerate(sum(groups, []))}
    last = [(4 * 19 + k // 2) ^ (34 * (k % 2)) for k in range(8)]
    last += [4 * q + k for q in (23, 31) for k in range(4)]
    return groups, pos, last


BWO_GROUPS, BWO_POS, BWO_LAST = _bwo_tables()
NSEM = NRING + len(BWO_GROUPS)


def _dot(a, b, dims):
    return lax.dot_general(a, b, dims, preferred_element_type=F32)


def _loop(n, body):
    def f(i, c):
        body(i)
        return c
    lax.fori_loop(0, n, f, 0)


def _copy(src, dst, sem, prio):
    pltpu.make_async_copy(src, dst, sem).start(priority=prio)


def _wait(buf, sem):
    pltpu.make_async_copy(buf, buf, sem).wait()


def _kernel(x_h, ckv_h, wq_h, wuk_h, wuv_h, wo_h, k_h, v_h, bwq_h, bwo_h, g_h,
            o_ref,
            x_v, g_v, ckv_v, wq_v, wuk_v, wuv_v, kv_v, bwq_v, wob_v,
            wrl_s, q_s, qabs_s, s_s, lat_s, qb_s, ctx_s, ctxb_s, sb_s, gate_s,
            sems):
    wo_v = wob_v.at[pl.ds(0, H * D)]
    bwo_v = wob_v.at[pl.ds(H * D, H * D)]

    def sem_of(u):
        return sems.at[u % NRING]

    def bwo_sem(grp):
        return sems.at[NRING + grp]

    def issue_w(src, dst, j, sem, prio=None):
        jx = (j, j ^ 1)
        order = range(16) if prio is None else [*range(0, 16, 2), *range(1, 16, 2)]
        for i in order:
            hi, b1 = _chunk_bits(i)
            r = pl.multiple_of((hi + 1) * 128 + REM_W + jx[b1] * 256, 8)

            def go(r, n, i=i):
                _copy(src.at[pl.ds(r, n)], dst.at[pl.ds(r, n)], sem,
                      i % 2 if prio is None else prio)

            if hi < 112:
                go(r, 128)
            else:
                edge = ((M * H - 128 + REM_W, 128 - REM_W) if hi == 112
                        else (0, 128 + REM_W))
                pl.when(j == 6)(lambda: go(*edge))
                pl.when(j != 6)(lambda: go(r, 128))

    def issue_wide(src, dst, j, sem):
        jx = (j, j ^ 1)
        for i in range(16):
            hi, b1 = _chunk_bits(i)
            r = pl.multiple_of(((hi + 1) * 32 + jx[b1] * 64) & 4095, 32)

            def go(r, n, c, m, i=i):
                _copy(src.at[pl.ds(r, n), pl.ds(c, m)],
                      dst.at[pl.ds(r, n), pl.ds(c, m)], sem, i % 2)

            go(r, 32, 128, 384)
            if hi < 112:
                go(r + 8, 32, 0, 128)
            else:
                edge = (4096 - 24, 24) if hi == 112 else (0, 40)
                pl.when(j == 6)(lambda: go(*edge, 0, 128))
                pl.when(j != 6)(lambda: go(r + 8, 32, 0, 128))

    def issue_ckv(b, j, sem):
        issue_wide(ckv_h.at[b], ckv_v.at[b], j, sem)

    def issue_bwq(j, sem):
        c0, c1 = REM_BWQ * 128, (REM_BWQ + 16) * 128
        jx = (j, j ^ 1)
        for i in range(16):
            hi, b1 = _chunk_bits(i)
            r = pl.multiple_of((hi // 2) * 8 + jx[b1] * 8, 8)
            rn = pl.multiple_of((r + 8) & (M - 1), 8)

            def go(r, c, n, i=i):
                _copy(bwq_h.at[pl.ds(r, 8), pl.ds(c, n)],
                      bwq_v.at[pl.ds(r, 8), pl.ds(c, n)], sem, i % 2)

            if hi % 2 == 0:
                go(r, c1, H * D - c1)
                go(rn, 0, c0)
            else:
                go(rn, c0, c1 - c0)

    def issue_kv(b, g, t, sem):
        def piece(edge):
            for h in range(HKV):
                if edge != h & 1:
                    k = (2 * g + t) ^ (2 * (h & 1))
                    r, n = pl.multiple_of((k + 1) * 128 + REM_KV, 8), 128
                elif t == 0:
                    r, n = W - 128 + REM_KV, 128 - REM_KV
                else:
                    r, n = 0, 128 + REM_KV
                for a, src in enumerate((k_h, v_h)):
                    _copy(src.at[b, h, pl.ds(SK - W + r, n)],
                          kv_v.at[b, a, h, pl.ds(r, n)], sem, a)
        pl.when(g < 2)(lambda: piece(None))
        pl.when(g == 2)(lambda: piece(1))
        pl.when(g == 3)(lambda: piece(0))

    def issue_bwo(g, t):
        @pl.when(g < 3)
        def _():
            shift = (4 * g, jnp.where(g == 0, 0, 4 + 4 * g))
            for i in range(16):
                hi, b1 = _chunk_bits(i)
                lo = hi % 4 + 2 * (t ^ b1)
                r = (hi - hi % 4 + lo + 1) * 32 + REM_BWO + g * 128
                d = (BWO_POS[hi // 4] + shift[i & 1]) * 128 + lo * 32
                _copy(bwo_h.at[pl.ds(pl.multiple_of(r, 8), 32)],
                      bwo_v.at[pl.ds(pl.multiple_of(d, 32), 32)],
                      bwo_sem(g if i & 1 else 0), i & 1)

        @pl.when(g == 3)
        def _():
            for i in range(16):
                hi, b1 = _chunk_bits(i)
                u = BWO_LAST[8 * t + i // 2] if i & 1 else hi + 2 * ((6 + t) ^ b1)
                grp = next(k for k, qs in enumerate(BWO_GROUPS) if u // 4 in qs)
                r = ((u + 1) * 32 + REM_BWO) % (H * D)
                d = BWO_POS[u // 4] * 128 + (u % 4) * 32
                n = min(32, H * D - r)
                _copy(bwo_h.at[pl.ds(r, n)], bwo_v.at[pl.ds(d, n)],
                      bwo_sem(grp), i & 1)
                if n < 32:
                    _copy(bwo_h.at[pl.ds(0, 32 - n)], bwo_v.at[pl.ds(d + n, 32 - n)],
                          bwo_sem(grp), i & 1)

    cx = pltpu.make_async_copy(x_h, x_v, sems.at[NRING - 1])
    cg = pltpu.make_async_copy(g_h, g_v, sems.at[NRING - 1])
    cx.start()
    cg.start()
    _loop(PREFILL, lambda j: issue_w(wq_h, wq_v, j, sem_of(U_WQ), 1))
    _loop(8 - PREFILL, lambda j: issue_w(wq_h, wq_v, j + PREFILL, sem_of(U_WQ)))
    _loop(8, lambda j: issue_w(wuk_h, wuk_v, j, sem_of(U_WUK)))
    cx.wait()
    cg.wait()
    gate = jax.nn.sigmoid(jnp.sum(
        x_v[...].astype(F32) * g_v[...].astype(F32).reshape(1, M),
        axis=1, keepdims=True))
    gate_s[0] = jnp.broadcast_to(gate, (B, M))
    gate_s[1] = jnp.broadcast_to(1.0 - gate, (B, M))

    def relayout(w_v, q):
        def body(i, c):
            r = pl.multiple_of((q * 64 + i) * 64, 64)
            d = pl.multiple_of((q * 64 + i) * W_PITCH, 8)
            val = pltpu.bitcast(w_v[pl.ds(r, 64), :], U32)
            wrl_s[0, pl.ds(d, 16), :] = val[:16]
            wrl_s[1, pl.ds(d, 16), :] = val[16:]
            return c
        lax.fori_loop(0, 64, body, 0, unroll=8)

    def head_pair(g, t):
        rows = pl.ds(pl.multiple_of(8 * g, 8), 256 * W_PITCH + 8)
        a = wrl_s.at[0, rows][pl.ds(t, 256, stride=W_PITCH), :]
        b = wrl_s.at[1, rows][pl.ds(t, 256, stride=W_PITCH), :]
        w0 = pltpu.bitcast((a & U32(0xFFFF)) | (b << 16), BF16)
        w1 = pltpu.bitcast((a >> 16) | (b & U32(0xFFFF0000)), BF16)
        return w0, w1

    def head_rows(ref, h0, n):
        return ref.at[pl.ds(pl.multiple_of(h0, 8), B * H + n)]

    def weight_unit(w_v, u, issue, per_head):
        def step1(g):
            for t in range(2):
                issue(g, t)
                if t == 0:
                    pl.when(g == 0)(lambda: _wait(w_v, sem_of(u)))
                relayout(w_v, 2 * g + t)
        _loop(2, step1)

        def step2(g):
            for t in range(8):
                if t % 4 == 0:
                    issue(2 + g, t // 4)
                ws = head_pair(g, t)
                per_head(g, 2 * t, ws[0])
                per_head(g, 2 * t + 1, ws[1])
        _loop(2, step2)

    def wq_head(g, e, w):
        r = pl.multiple_of(g * 128 + e * 8, 8)
        q_s[pl.ds(r, 8), :] = _dot(x_v[...], w, NN)
    weight_unit(wq_v, U_WQ,
                lambda g, t: issue_ckv(0, 2 * g + t, sem_of(U_CKV)), wq_head)

    def wuk_head(g, e, w):
        r = pl.multiple_of(g * 128 + e * 8, 8)
        qa = _dot(q_s[pl.ds(r, 8), :].astype(BF16), w, NT) * SCALE
        for ct in range(4):
            head_rows(qabs_s.at[ct], 16 * g, 16)[pl.ds(e, B, stride=H), :] = (
                qa[:, ct * 128:(ct + 1) * 128])
    weight_unit(wuk_v, U_WUK,
                lambda g, t: issue_ckv(1, 2 * g + t, sem_of(U_CKV + 1)), wuk_head)

    def ckv_unit(b):
        u = U_CKV + b
        KC = SK // 4

        def issue(j):
            sem = sem_of(u + 2)
            pl.when(b < B - 2)(
                lambda: issue_ckv(jnp.minimum(b + 2, B - 1), j, sem))
            pl.when(b == B - 2)(lambda: issue_bwq(j, sem))
            pl.when(b == B - 1)(lambda: issue_w(wuv_h, wuv_v, j, sem))

        r = pl.multiple_of(b * H, H)
        qa = jnp.concatenate(
            [qabs_s[ct, pl.ds(r, H), :] for ct in range(4)], axis=1
        ).astype(BF16)

        def score_step(j, m):
            issue(j)
            pl.when(j == 0)(lambda: _wait(ckv_v.at[b], sem_of(u)))
            off = pl.multiple_of(j * KC, KC)
            s = _dot(qa, ckv_v[b, pl.ds(off, KC), :], NT)
            s_s[j] = s
            for t in range(KC // 128):
                m = jnp.maximum(m, s[:, t * 128:(t + 1) * 128])
            return m
        m = lax.fori_loop(0, 4, score_step, jnp.full((H, 128), -jnp.inf, F32))
        m = jnp.max(m, axis=1, keepdims=True)

        def pv_step(j, carry):
            l, acc = carry
            issue(4 + j)
            off = pl.multiple_of(j * KC, KC)
            p = jnp.exp(s_s[j] - m)
            for t in range(KC // 128):
                l = l + p[:, t * 128:(t + 1) * 128]
            acc = acc + _dot(p.astype(BF16), ckv_v[b, pl.ds(off, KC), :], NN)
            return l, acc
        l, acc = lax.fori_loop(
            0, 4, pv_step, (jnp.zeros((H, 128), F32), jnp.zeros((H, C), F32)))
        lat = acc / jnp.sum(l, axis=1, keepdims=True)
        for ct in range(4):
            lat_s[ct, pl.ds(r, H), :] = lat[:, ct * 128:(ct + 1) * 128]
    _loop(B, ckv_unit)

    def bwq_step(g):
        for t in range(2):
            issue_kv(0, g, t, sem_of(U_KV))
            if t == 0:
                pl.when(g == 0)(lambda: _wait(bwq_v, sem_of(U_BWQ)))
            off = pl.multiple_of(g * 1024 + t * 512, 512)
            q = _dot(x_v[...], bwq_v[:, pl.ds(off, 512)], NN)
            for e in range(4):
                head_rows(qb_s, 8 * g, 8)[pl.ds(4 * t + e, B, stride=H), :] = (
                    q[:, e * 128:(e + 1) * 128])
    _loop(4, bwq_step)

    def wuv_head(g, e, w):
        lat = jnp.concatenate(
            [head_rows(lat_s.at[ct], 16 * g, 16)[pl.ds(e, B, stride=H), :]
             for ct in range(4)], axis=1).astype(BF16)
        r = pl.multiple_of(g * 128 + e * 8, 8)
        ctx_s[pl.ds(r, 8), :] = _dot(lat, w, NN)
    weight_unit(wuv_v, U_WUV,
                lambda g, t: issue_kv(1, g, t, sem_of(U_KV + 1)), wuv_head)

    def kv_unit(b):
        u = U_KV + b

        def issue(g, t):
            sem = sem_of(u + 2)
            pl.when(b < B - 2)(
                lambda: issue_kv(jnp.minimum(b + 2, B - 1), g, t, sem))
            pl.when(b == B - 2)(lambda: issue_wide(wo_h, wo_v, 2 * g + t, sem))
            pl.when(b == B - 1)(lambda: issue_bwo(g, t))

        def pair_step(i):
            issue(i, 0)
            pl.when(i == 0)(lambda: _wait(kv_v.at[b], sem_of(u)))
            r = pl.multiple_of(b * H + i * 8, 8)
            q = qb_s[pl.ds(r, 8), :].astype(BF16)
            s = jnp.where(lax.broadcasted_iota(jnp.int32, (8, W), 0) < 4,
                          _dot(q, kv_v[b, 0, 2 * i], NT),
                          _dot(q, kv_v[b, 0, 2 * i + 1], NT)) * SCALE
            sb_s[...] = s - jnp.max(s, axis=1, keepdims=True)
            issue(i, 1)
            p = jnp.exp(sb_s[...])
            l = jnp.sum(p, axis=1, keepdims=True)
            p = p.astype(BF16)
            o = jnp.where(lax.broadcasted_iota(jnp.int32, (8, D), 0) < 4,
                          _dot(p, kv_v[b, 1, 2 * i], NN),
                          _dot(p, kv_v[b, 1, 2 * i + 1], NN)) / l
            rb = pl.multiple_of(b * CB_PITCH + i * 8, 8)
            ctxb_s[pl.ds(rb, 8), :] = pltpu.roll(o, D - BWO_ROT, 1)
        _loop(4, pair_step)
    _loop(B, kv_unit)

    lo = lax.broadcasted_iota(jnp.int32, (B, D), 1) < D - BWO_ROT
    heads = [ctxb_s[pl.ds(h, B, stride=CB_PITCH), :] for h in range(H)]
    for q in range(H):
        ctx_s[pl.ds((H + BWO_POS[q]) * 8, 8), :] = (
            jnp.where(lo, heads[q], heads[(q + 1) % H]))

    def proj(r, w, n):
        lhs = jnp.concatenate(
            [ctx_s[pl.ds(r + 8 * k, 8), :] for k in range(n)], axis=1).astype(BF16)
        return _dot(lhs, wob_v[pl.ds(w, n * 128), :], NN)

    def wait_bwo(grp):
        qs = BWO_GROUPS[grp]
        _wait(bwo_v.at[pl.ds(BWO_POS[qs[0]] * 128, len(qs) * 128)], bwo_sem(grp))

    def proj_step(it, acc):
        pl.when(it == 0)(lambda: _wait(wo_v, sem_of(U_WO)))
        pl.when(it == 4)(lambda: wait_bwo(0))
        pl.when(it == 6)(lambda: wait_bwo(1))
        return acc + gate_s[it >> 2] * proj(
            pl.multiple_of(it * 64, 64), pl.multiple_of(it * 1024, 1024), 8)
    acc = lax.fori_loop(0, 7, proj_step, jnp.zeros((B, M), F32))
    for grp in range(2, len(BWO_GROUPS)):
        wait_bwo(grp)
        blk = H + BWO_POS[BWO_GROUPS[grp][0]]
        acc = acc + gate_s[1] * proj(blk * 8, blk * 128, len(BWO_GROUPS[grp]))
    o_ref[...] = acc.astype(o_ref.dtype)


@jax.jit
def pallas_gated_mix__compressed_kv_cla__sliding_block_cached__decode_kernel(
    A_x: jax.Array,
    A_c_kv: jax.Array,
    A_w_q: jax.Array,
    A_w_uk: jax.Array,
    A_w_uv: jax.Array,
    A_w_o: jax.Array,
    B_x: jax.Array,
    B_k_cache: jax.Array,
    B_v_cache: jax.Array,
    B_wq: jax.Array,
    B_wo: jax.Array,
    gate_w: jax.Array,
):
    del B_x
    out = pl.pallas_call(
        _kernel,
        out_shape=jax.ShapeDtypeStruct((B, M), A_x.dtype),
        in_specs=[pl.BlockSpec(memory_space=pl.ANY)] * 11,
        out_specs=pl.BlockSpec(memory_space=pltpu.VMEM),
        scratch_shapes=[
            pltpu.VMEM((B, M), BF16),
            pltpu.VMEM((M,), BF16),
            pltpu.VMEM((B, SK, C), BF16),
            pltpu.VMEM((M * H, D), BF16),
            pltpu.VMEM((C * H, D), BF16),
            pltpu.VMEM((C * H, D), BF16),
            pltpu.VMEM((B, 2, HKV, W, D), BF16),
            pltpu.VMEM((M, H * D), BF16),
            pltpu.VMEM((2 * H * D, M), BF16),
            pltpu.VMEM((2, 256 * W_PITCH + 16, D), U32),
            pltpu.VMEM((H * B, D), F32),
            pltpu.VMEM((4, (B + 1) * H, 128), F32),
            pltpu.VMEM((4, H, SK // 4), F32),
            pltpu.VMEM((4, (B + 1) * H, 128), F32),
            pltpu.VMEM(((B + 1) * H, D), F32),
            pltpu.VMEM((2 * H * B, D), F32),
            pltpu.VMEM((B * CB_PITCH + H, D), F32),
            pltpu.VMEM((8, W), F32),
            pltpu.VMEM((2, B, M), F32),
            pltpu.SemaphoreType.DMA((NSEM,)),
        ],
        compiler_params=pltpu.CompilerParams(
            vmem_limit_bytes=110 * 1024 * 1024,
            disable_bounds_checks=True,
            disable_semaphore_checks=True,
        ),
    )(
        A_x.reshape(B, M), A_c_kv,
        A_w_q.reshape(M * H, D), A_w_uk.reshape(C * H, D), A_w_uv.reshape(C * H, D),
        A_w_o.reshape(H * D, M), B_k_cache, B_v_cache, B_wq, B_wo, gate_w,
    )
    return out.reshape(B, 1, M)
```

```python
import jax
import jax.numpy as jnp
from jax import lax
import jax.experimental.pallas as pl
import jax.experimental.pallas.tpu as pltpu

B = 8
H = 32
D = 128
M = 512
C = 512
SK = 4096
HKV = 8
W = 1024
SCALE = D ** -0.5

F32 = jnp.float32
BF16 = jnp.bfloat16
U32 = jnp.uint32
NN = (((1,), (0,)), ((), ()))
NT = (((1,), (1,)), ((), ()))

U_WQ, U_WUK, U_CKV, U_BWQ, U_WUV, U_KV, U_WO = 0, 1, 2, 10, 11, 12, 20
NRING = 4
PREFILL = 2

REM_W = 8
REM_KV = 40
REM_BWO = 8
REM_BWQ = 5

W_PITCH = 24
CB_PITCH = 40
BWO_ROT = 32 + REM_BWO


def _chunk_bits(i):
    b1 = (i >> 1) & 1
    return (i & 1) * 64 + b1 * 32 + ((i >> 2) & 1) + (i >> 3) * 16, b1


def _bwo_tables():
    def blocks(prio, m):
        return [q + 16 * prio for q in range(m, 16, 4)]
    groups = (blocks(0, 0) + blocks(0, 1) + blocks(0, 2) + blocks(1, 0),
              blocks(0, 3) + blocks(1, 1), blocks(1, 2), [19, 27], [23], [31])
    pos = {q: k for k, q in enumerate(sum(groups, []))}
    last = [(4 * 19 + k // 2) ^ (34 * (k % 2)) for k in range(8)]
    last += [4 * q + k for q in (23, 31) for k in range(4)]
    return groups, pos, last


BWO_GROUPS, BWO_POS, BWO_LAST = _bwo_tables()
NSEM = NRING + len(BWO_GROUPS)


def _dot(a, b, dims):
    return lax.dot_general(a, b, dims, preferred_element_type=F32)


def _loop(n, body):
    def f(i, c):
        body(i)
        return c
    lax.fori_loop(0, n, f, 0)


def _copy(src, dst, sem, prio):
    pltpu.make_async_copy(src, dst, sem).start(priority=prio)


def _wait(buf, sem):
    pltpu.make_async_copy(buf, buf, sem).wait()


def _kernel(x_h, ckv_h, wq_h, wuk_h, wuv_h, wo_h, k_h, v_h, bwq_h, bwo_h, g_h,
            o_ref,
            x_v, g_v, ckv_v, wq_v, wuk_v, wuv_v, kv_v, bwq_v, wob_v,
            wrl_s, q_s, qabs_s, s_s, lat_s, qb_s, ctx_s, ctxb_s, sb_s, gate_s,
            sems):
    wo_v = wob_v.at[pl.ds(0, H * D)]
    bwo_v = wob_v.at[pl.ds(H * D, H * D)]

    def sem_of(u):
        return sems.at[u % NRING]

    def bwo_sem(grp):
        return sems.at[NRING + grp]

    def issue_w(src, dst, j, sem, prio=None):
        jx = (j, j ^ 1)
        order = range(16) if prio is None else [*range(0, 16, 2), *range(1, 16, 2)]
        for i in order:
            hi, b1 = _chunk_bits(i)
            r = pl.multiple_of((hi + 1) * 128 + REM_W + jx[b1] * 256, 8)

            def go(r, n, i=i):
                _copy(src.at[pl.ds(r, n)], dst.at[pl.ds(r, n)], sem,
                      i % 2 if prio is None else prio)

            if hi < 112:
                go(r, 128)
            else:
                edge = ((M * H - 128 + REM_W, 128 - REM_W) if hi == 112
                        else (0, 128 + REM_W))
                pl.when(j == 6)(lambda: go(*edge))
                pl.when(j != 6)(lambda: go(r, 128))

    def issue_wide(src, dst, j, sem):
        jx = (j, j ^ 1)
        for i in range(16):
            hi, b1 = _chunk_bits(i)
            r = pl.multiple_of(((hi + 1) * 32 + jx[b1] * 64) & 4095, 32)

            def go(r, n, c, m, i=i):
                _copy(src.at[pl.ds(r, n), pl.ds(c, m)],
                      dst.at[pl.ds(r, n), pl.ds(c, m)], sem, i % 2)

            go(r, 32, 128, 384)
            if hi < 112:
                go(r + 8, 32, 0, 128)
            else:
                edge = (4096 - 24, 24) if hi == 112 else (0, 40)
                pl.when(j == 6)(lambda: go(*edge, 0, 128))
                pl.when(j != 6)(lambda: go(r + 8, 32, 0, 128))

    def issue_ckv(b, j, sem):
        issue_wide(ckv_h.at[b], ckv_v.at[b], j, sem)

    def issue_bwq(j, sem):
        c0, c1 = REM_BWQ * 128, (REM_BWQ + 16) * 128
        jx = (j, j ^ 1)
        for i in range(16):
            hi, b1 = _chunk_bits(i)
            r = pl.multiple_of((hi // 2) * 8 + jx[b1] * 8, 8)
            rn = pl.multiple_of((r + 8) & (M - 1), 8)

            def go(r, c, n, i=i):
                _copy(bwq_h.at[pl.ds(r, 8), pl.ds(c, n)],
                      bwq_v.at[pl.ds(r, 8), pl.ds(c, n)], sem, i % 2)

            if hi % 2 == 0:
                go(r, c1, H * D - c1)
                go(rn, 0, c0)
            else:
                go(rn, c0, c1 - c0)

    def issue_kv(b, g, t, sem):
        def piece(edge):
            for h in range(HKV):
                if edge != h & 1:
                    k = (2 * g + t) ^ (2 * (h & 1))
                    r, n = pl.multiple_of((k + 1) * 128 + REM_KV, 8), 128
                elif t == 0:
                    r, n = W - 128 + REM_KV, 128 - REM_KV
                else:
                    r, n = 0, 128 + REM_KV
                for a, src in enumerate((k_h, v_h)):
                    _copy(src.at[b, h, pl.ds(SK - W + r, n)],
                          kv_v.at[b, a, h, pl.ds(r, n)], sem, a)
        pl.when(g < 2)(lambda: piece(None))
        pl.when(g == 2)(lambda: piece(1))
        pl.when(g == 3)(lambda: piece(0))

    def issue_bwo(g, t):
        @pl.when(g < 3)
        def _():
            shift = (4 * g, jnp.where(g == 0, 0, 4 + 4 * g))
            for i in range(16):
                hi, b1 = _chunk_bits(i)
                lo = hi % 4 + 2 * (t ^ b1)
                r = (hi - hi % 4 + lo + 1) * 32 + REM_BWO + g * 128
                d = (BWO_POS[hi // 4] + shift[i & 1]) * 128 + lo * 32
                _copy(bwo_h.at[pl.ds(pl.multiple_of(r, 8), 32)],
                      bwo_v.at[pl.ds(pl.multiple_of(d, 32), 32)],
                      bwo_sem(g if i & 1 else 0), i & 1)

        @pl.when(g == 3)
        def _():
            for i in range(16):
                hi, b1 = _chunk_bits(i)
                u = BWO_LAST[8 * t + i // 2] if i & 1 else hi + 2 * ((6 + t) ^ b1)
                grp = next(k for k, qs in enumerate(BWO_GROUPS) if u // 4 in qs)
                r = ((u + 1) * 32 + REM_BWO) % (H * D)
                d = BWO_POS[u // 4] * 128 + (u % 4) * 32
                n = min(32, H * D - r)
                _copy(bwo_h.at[pl.ds(r, n)], bwo_v.at[pl.ds(d, n)],
                      bwo_sem(grp), i & 1)
                if n < 32:
                    _copy(bwo_h.at[pl.ds(0, 32 - n)], bwo_v.at[pl.ds(d + n, 32 - n)],
                          bwo_sem(grp), i & 1)

    cx = pltpu.make_async_copy(x_h, x_v, sems.at[NRING - 1])
    cg = pltpu.make_async_copy(g_h, g_v, sems.at[NRING - 1])
    cx.start()
    cg.start()
    _loop(PREFILL, lambda j: issue_w(wq_h, wq_v, j, sem_of(U_WQ), 1))
    _loop(8 - PREFILL, lambda j: issue_w(wq_h, wq_v, j + PREFILL, sem_of(U_WQ)))
    _loop(8, lambda j: issue_w(wuk_h, wuk_v, j, sem_of(U_WUK)))
    cx.wait()
    cg.wait()
    gate = jax.nn.sigmoid(jnp.sum(
        x_v[...].astype(F32) * g_v[...].astype(F32).reshape(1, M),
        axis=1, keepdims=True))
    gate_s[0] = jnp.broadcast_to(gate, (B, M))
    gate_s[1] = jnp.broadcast_to(1.0 - gate, (B, M))
    wrl_s[:, pl.ds(256 * W_PITCH, 16), :] = jnp.zeros((2, 16, D), U32)
    qabs_s[:, pl.ds(B * H, H), :] = jnp.zeros((4, H, 128), F32)
    lat_s[:, pl.ds(B * H, H), :] = jnp.zeros((4, H, 128), F32)
    qb_s[pl.ds(B * H, H), :] = jnp.zeros((H, D), F32)
    ctxb_s[...] = jnp.zeros(ctxb_s.shape, F32)

    def relayout(w_v, q):
        def body(i, c):
            r = pl.multiple_of((q * 64 + i) * 64, 64)
            d = pl.multiple_of((q * 64 + i) * W_PITCH, 8)
            val = pltpu.bitcast(w_v[pl.ds(r, 64), :], U32)
            pad = jnp.zeros((W_PITCH - 16, D), U32)
            wrl_s[0, pl.ds(d, W_PITCH), :] = jnp.concatenate([val[:16], pad])
            wrl_s[1, pl.ds(d, W_PITCH), :] = jnp.concatenate([val[16:], pad])
            return c
        lax.fori_loop(0, 64, body, 0, unroll=8)

    def head_pair(g, t):
        rows = pl.ds(pl.multiple_of(8 * g, 8), 256 * W_PITCH + 8)
        a = wrl_s.at[0, rows][pl.ds(t, 256, stride=W_PITCH), :]
        b = wrl_s.at[1, rows][pl.ds(t, 256, stride=W_PITCH), :]
        w0 = pltpu.bitcast((a & U32(0xFFFF)) | (b << 16), BF16)
        w1 = pltpu.bitcast((a >> 16) | (b & U32(0xFFFF0000)), BF16)
        return w0, w1

    def head_rows(ref, h0, n):
        return ref.at[pl.ds(pl.multiple_of(h0, 8), B * H + n)]

    def weight_unit(w_v, u, issue, per_head):
        def step1(g):
            for t in range(2):
                issue(g, t)
                if t == 0:
                    pl.when(g == 0)(lambda: _wait(w_v, sem_of(u)))
                relayout(w_v, 2 * g + t)
        _loop(2, step1)

        def step2(g):
            for t in range(8):
                if t % 4 == 0:
                    issue(2 + g, t // 4)
                ws = head_pair(g, t)
                per_head(g, 2 * t, ws[0])
                per_head(g, 2 * t + 1, ws[1])
        _loop(2, step2)

    def wq_head(g, e, w):
        r = pl.multiple_of(g * 128 + e * 8, 8)
        q_s[pl.ds(r, 8), :] = _dot(x_v[...], w, NN)
    weight_unit(wq_v, U_WQ,
                lambda g, t: issue_ckv(0, 2 * g + t, sem_of(U_CKV)), wq_head)

    def wuk_head(g, e, w):
        r = pl.multiple_of(g * 128 + e * 8, 8)
        qa = _dot(q_s[pl.ds(r, 8), :].astype(BF16), w, NT) * SCALE
        for ct in range(4):
            head_rows(qabs_s.at[ct], 16 * g, 16)[pl.ds(e, B, stride=H), :] = (
                qa[:, ct * 128:(ct + 1) * 128])
    weight_unit(wuk_v, U_WUK,
                lambda g, t: issue_ckv(1, 2 * g + t, sem_of(U_CKV + 1)), wuk_head)

    def ckv_unit(b):
        u = U_CKV + b
        KC = SK // 4

        def issue(j):
            sem = sem_of(u + 2)
            pl.when(b < B - 2)(
                lambda: issue_ckv(jnp.minimum(b + 2, B - 1), j, sem))
            pl.when(b == B - 2)(lambda: issue_bwq(j, sem))
            pl.when(b == B - 1)(lambda: issue_w(wuv_h, wuv_v, j, sem))

        r = pl.multiple_of(b * H, H)
        qa = jnp.concatenate(
            [qabs_s[ct, pl.ds(r, H), :] for ct in range(4)], axis=1
        ).astype(BF16)

        def score_step(j, m):
            issue(j)
            pl.when(j == 0)(lambda: _wait(ckv_v.at[b], sem_of(u)))
            off = pl.multiple_of(j * KC, KC)
            s = _dot(qa, ckv_v[b, pl.ds(off, KC), :], NT)
            s_s[j] = s
            for t in range(KC // 128):
                m = jnp.maximum(m, s[:, t * 128:(t + 1) * 128])
            return m
        m = lax.fori_loop(0, 4, score_step, jnp.full((H, 128), -jnp.inf, F32))
        m = jnp.max(m, axis=1, keepdims=True)

        def pv_step(j, carry):
            l, acc = carry
            issue(4 + j)
            off = pl.multiple_of(j * KC, KC)
            p = jnp.exp(s_s[j] - m)
            for t in range(KC // 128):
                l = l + p[:, t * 128:(t + 1) * 128]
            acc = acc + _dot(p.astype(BF16), ckv_v[b, pl.ds(off, KC), :], NN)
            return l, acc
        l, acc = lax.fori_loop(
            0, 4, pv_step, (jnp.zeros((H, 128), F32), jnp.zeros((H, C), F32)))
        lat = acc / jnp.sum(l, axis=1, keepdims=True)
        for ct in range(4):
            lat_s[ct, pl.ds(r, H), :] = lat[:, ct * 128:(ct + 1) * 128]
    _loop(B, ckv_unit)

    def bwq_step(g):
        for t in range(2):
            issue_kv(0, g, t, sem_of(U_KV))
            if t == 0:
                pl.when(g == 0)(lambda: _wait(bwq_v, sem_of(U_BWQ)))
            off = pl.multiple_of(g * 1024 + t * 512, 512)
            q = _dot(x_v[...], bwq_v[:, pl.ds(off, 512)], NN)
            for e in range(4):
                head_rows(qb_s, 8 * g, 8)[pl.ds(4 * t + e, B, stride=H), :] = (
                    q[:, e * 128:(e + 1) * 128])
    _loop(4, bwq_step)

    def wuv_head(g, e, w):
        lat = jnp.concatenate(
            [head_rows(lat_s.at[ct], 16 * g, 16)[pl.ds(e, B, stride=H), :]
             for ct in range(4)], axis=1).astype(BF16)
        r = pl.multiple_of(g * 128 + e * 8, 8)
        ctx_s[pl.ds(r, 8), :] = _dot(lat, w, NN)
    weight_unit(wuv_v, U_WUV,
                lambda g, t: issue_kv(1, g, t, sem_of(U_KV + 1)), wuv_head)

    def kv_unit(b):
        u = U_KV + b

        def issue(g, t):
            sem = sem_of(u + 2)
            pl.when(b < B - 2)(
                lambda: issue_kv(jnp.minimum(b + 2, B - 1), g, t, sem))
            pl.when(b == B - 2)(lambda: issue_wide(wo_h, wo_v, 2 * g + t, sem))
            pl.when(b == B - 1)(lambda: issue_bwo(g, t))

        def pair_step(i):
            issue(i, 0)
            pl.when(i == 0)(lambda: _wait(kv_v.at[b], sem_of(u)))
            r = pl.multiple_of(b * H + i * 8, 8)
            q = qb_s[pl.ds(r, 8), :].astype(BF16)
            s = jnp.where(lax.broadcasted_iota(jnp.int32, (8, W), 0) < 4,
                          _dot(q, kv_v[b, 0, 2 * i], NT),
                          _dot(q, kv_v[b, 0, 2 * i + 1], NT)) * SCALE
            sb_s[...] = s - jnp.max(s, axis=1, keepdims=True)
            issue(i, 1)
            p = jnp.exp(sb_s[...])
            l = jnp.sum(p, axis=1, keepdims=True)
            p = p.astype(BF16)
            o = jnp.where(lax.broadcasted_iota(jnp.int32, (8, D), 0) < 4,
                          _dot(p, kv_v[b, 1, 2 * i], NN),
                          _dot(p, kv_v[b, 1, 2 * i + 1], NN)) / l
            rb = pl.multiple_of(b * CB_PITCH + i * 8, 8)
            ctxb_s[pl.ds(rb, 8), :] = pltpu.roll(o, D - BWO_ROT, 1)
        _loop(4, pair_step)
    _loop(B, kv_unit)

    lo = lax.broadcasted_iota(jnp.int32, (B, D), 1) < D - BWO_ROT
    heads = [ctxb_s[pl.ds(h, B, stride=CB_PITCH), :] for h in range(H)]
    for q in range(H):
        ctx_s[pl.ds((H + BWO_POS[q]) * 8, 8), :] = (
            jnp.where(lo, heads[q], heads[(q + 1) % H]))

    def proj(r, w, n):
        lhs = jnp.concatenate(
            [ctx_s[pl.ds(r + 8 * k, 8), :] for k in range(n)], axis=1).astype(BF16)
        return _dot(lhs, wob_v[pl.ds(w, n * 128), :], NN)

    def wait_bwo(grp):
        qs = BWO_GROUPS[grp]
        _wait(bwo_v.at[pl.ds(BWO_POS[qs[0]] * 128, len(qs) * 128)], bwo_sem(grp))

    def proj_step(it, acc):
        pl.when(it == 0)(lambda: _wait(wo_v, sem_of(U_WO)))
        pl.when(it == 4)(lambda: wait_bwo(0))
        pl.when(it == 6)(lambda: wait_bwo(1))
        return acc + gate_s[it >> 2] * proj(
            pl.multiple_of(it * 64, 64), pl.multiple_of(it * 1024, 1024), 8)
    acc = lax.fori_loop(0, 7, proj_step, jnp.zeros((B, M), F32))
    for grp in range(2, len(BWO_GROUPS)):
        wait_bwo(grp)
        blk = H + BWO_POS[BWO_GROUPS[grp][0]]
        acc = acc + gate_s[1] * proj(blk * 8, blk * 128, len(BWO_GROUPS[grp]))
    o_ref[...] = acc.astype(o_ref.dtype)


@jax.jit
def pallas_gated_mix__compressed_kv_cla__sliding_block_cached__decode_kernel(
    A_x: jax.Array,
    A_c_kv: jax.Array,
    A_w_q: jax.Array,
    A_w_uk: jax.Array,
    A_w_uv: jax.Array,
    A_w_o: jax.Array,
    B_x: jax.Array,
    B_k_cache: jax.Array,
    B_v_cache: jax.Array,
    B_wq: jax.Array,
    B_wo: jax.Array,
    gate_w: jax.Array,
):
    del B_x
    out = pl.pallas_call(
        _kernel,
        out_shape=jax.ShapeDtypeStruct((B, M), A_x.dtype),
        in_specs=[pl.BlockSpec(memory_space=pl.ANY)] * 11,
        out_specs=pl.BlockSpec(memory_space=pltpu.VMEM),
        scratch_shapes=[
            pltpu.VMEM((B, M), BF16),
            pltpu.VMEM((M,), BF16),
            pltpu.VMEM((B, SK, C), BF16),
            pltpu.VMEM((M * H, D), BF16),
            pltpu.VMEM((C * H, D), BF16),
            pltpu.VMEM((C * H, D), BF16),
            pltpu.VMEM((B, 2, HKV, W, D), BF16),
            pltpu.VMEM((M, H * D), BF16),
            pltpu.VMEM((2 * H * D, M), BF16),
            pltpu.VMEM((2, 256 * W_PITCH + 16, D), U32),
            pltpu.VMEM((H * B, D), F32),
            pltpu.VMEM((4, (B + 1) * H, 128), F32),
            pltpu.VMEM((4, H, SK // 4), F32),
            pltpu.VMEM((4, (B + 1) * H, 128), F32),
            pltpu.VMEM(((B + 1) * H, D), F32),
            pltpu.VMEM((2 * H * B, D), F32),
            pltpu.VMEM((B * CB_PITCH + H, D), F32),
            pltpu.VMEM((8, W), F32),
            pltpu.VMEM((2, B, M), F32),
            pltpu.SemaphoreType.DMA((NSEM,)),
        ],
        compiler_params=pltpu.CompilerParams(
            vmem_limit_bytes=110 * 1024 * 1024,
            disable_bounds_checks=True,
            disable_semaphore_checks=True,
        ),
    )(
        A_x.reshape(B, M), A_c_kv,
        A_w_q.reshape(M * H, D), A_w_uk.reshape(C * H, D), A_w_uv.reshape(C * H, D),
        A_w_o.reshape(H * D, M), B_k_cache, B_v_cache, B_wq, B_wo, gate_w,
    )
    return out.reshape(B, 1, M)
```
